```python
import os as _os
_os.environ.setdefault('JAX_PLATFORMS', 'cpu')
import jax
import jax.numpy as jnp

def _softmax(x, axis=-1):
    return jax.nn.softmax(x, axis=axis)

def _gelu(x):
    return jax.nn.gelu(x, approximate=True)

def _silu(x):
    return jax.nn.silu(x)

def _sigmoid(x):
    return jax.nn.sigmoid(x)

def _layernorm(x, axis=-1, eps=1e-05):
    m = jnp.mean(x, axis=axis, keepdims=True)
    v = jnp.var(x, axis=axis, keepdims=True)
    return (x - m) / jnp.sqrt(v + eps)

def _scatter_add(tgt, idx, src, axis=0):
    return tgt.at[idx].add(src)

def _segment_sum(src, seg, n):
    return jax.ops.segment_sum(src, seg, n)

class _Rng:

    def __init__(self, key):
        self._k = key

    def _next(self):
        self._k, sub = jax.random.split(self._k)
        return sub

    def normal(self, shape):
        return jax.random.normal(self._next(), shape, dtype=jnp.bfloat16)

    def randint(self, lo, hi, shape):
        return jax.random.randint(self._next(), shape, lo, hi, dtype=jnp.int32)

    def uniform(self, shape, lo=0.0, hi=1.0):
        return jax.random.uniform(self._next(), shape, jnp.bfloat16, lo, hi)

    def permutation(self, n):
        return jax.random.permutation(self._next(), n)
kernel_name = 'concat_heads__spectral_gfnet__memory_aug_recurrent_mem_tr__prompt'

def setup_inputs():
    _rng = _Rng(jax.random.key(int.from_bytes(__import__("os").urandom(4), "little")))
    _w = lambda a: (lambda t: t.astype(jnp.bfloat16) if jnp.issubdtype(t.dtype, jnp.floating) else t)(jnp.asarray(a))

    def _A_setup():
        B, S, D = (1, 2048, 512)
        Df = D // 2 + 1
        return {'x': _w((lambda *s: _rng.normal(s) * 0.05)(B, S, D)), 'w_r': _w((lambda *s: _rng.normal(s) * 0.05)(S, Df) * 0.02), 'w_i': _w((lambda *s: _rng.normal(s) * 0.05)(S, Df) * 0.02)}
    _A_in = _A_setup()

    def _B_setup():
        B, S, Dm = (1, 2048, 512)
        H, Dh = (32, 128)
        M, seg = (8, 32)
        seg = min(seg, S)
        S = S // seg * seg
        return {'x': _w((lambda *s: _rng.normal(s) * 0.05)(B, S, Dm)), 'mem0': _w((lambda *s: _rng.normal(s) * 0.4)(B, M, Dm)), 'Wq': _w((lambda *s: _rng.normal(s) * 3.2)(Dm, H, Dh) * Dm ** (-0.5)), 'Wk': _w((lambda *s: _rng.normal(s) * 3.2)(Dm, H, Dh) * Dm ** (-0.5)), 'Wv': _w((lambda *s: _rng.normal(s) * 0.4)(Dm, H, Dh) * Dm ** (-0.5)), 'Wo': _w((lambda *s: _rng.normal(s) * 0.4)(H, Dh, Dm) * (H * Dh) ** (-0.5)), 'seg_len': seg}
    _B_in = _B_setup()
    return {'A_x': _A_in['x'], 'A_w_r': _A_in['w_r'], 'A_w_i': _A_in['w_i'], 'B_x': _B_in['x'], 'B_mem0': _B_in['mem0'], 'B_Wq': _B_in['Wq'], 'B_Wk': _B_in['Wk'], 'B_Wv': _B_in['Wv'], 'B_Wo': _B_in['Wo'], 'B_seg_len': _B_in['seg_len']}

def reference(A_x, A_w_r, A_w_i, B_x, B_mem0, B_Wq, B_Wk, B_Wv, B_Wo, B_seg_len):

    def _A_ref(x, w_r, w_i):
        B, S, D = x.shape
        X = (lambda x, axes=(-2, -1): jnp.fft.rfft2(x.astype(jnp.float32), axes=axes))(x, axes=(-2, -1))
        W = w_r + 1j * w_i
        X = X * W
        y = (lambda x, s, axes=(-2, -1): jnp.fft.irfft2(x, s=s, axes=axes).astype(jnp.bfloat16))(X, (S, D), axes=(-2, -1))
        return y

    def _B_ref(x, mem0, Wq, Wk, Wv, Wo, seg_len):
        B, S, Dm = x.shape
        H, Dh = (Wq.shape[1], Wq.shape[2])
        M = mem0.shape[1]
        scale = Dh ** (-0.5)
        n_seg = S // seg_len
        L = M + seg_len
        idx = jnp.arange(L)
        mask = (idx[:, None] < M) | (idx[:, None] >= idx[None, :])
        mem = mem0
        outs = []
        for s in range(n_seg):
            xs = x[:, s * seg_len:(s + 1) * seg_len, :].copy()
            h = jnp.concatenate([mem, xs], axis=1)
            q = jnp.einsum('btd,dhe->bhte', h, Wq)
            k = jnp.einsum('btd,dhe->bhte', h, Wk)
            v = jnp.einsum('btd,dhe->bhte', h, Wv)
            scores = jnp.einsum('bhqe,bhke->bhqk', q, k) * scale
            scores = jnp.where(mask[None, None], scores, -1000000000.0)
            p = _softmax(scores, axis=-1)
            o = jnp.einsum('bhqk,bhke->bhqe', p, v)
            o = jnp.einsum('bhte,hed->btd', o, Wo)
            mem = o[:, :M, :].copy()
            outs.append(o[:, M:, :])
        return jnp.concatenate(outs, axis=1)
    a = _A_ref(A_x, A_w_r, A_w_i)
    b = _B_ref(B_x, B_mem0, B_Wq, B_Wk, B_Wv, B_Wo, B_seg_len)
    return jnp.concatenate([a, b], axis=-1)
```

```python
import functools

import jax
import jax.numpy as jnp
import numpy as np
from jax import lax
from jax.experimental import pallas as pl
from jax.experimental.pallas import tpu as pltpu

F32, BF16, U32 = jnp.float32, jnp.bfloat16, jnp.uint32

S, D = 2048, 512
H, DH, M, SEG = 32, 128, 8, 32
L = M + SEG
NSEG = S // SEG
N1, N2 = 32, 64
R0, RX = 512, 24
RING = 576
XP, YP, WP = 17, 33, 257
LOG2E = 1.4426950408889634
UNIT = 8 * WP + 8
A_WQKV = 0
A_WO = A_WQKV + 12 * UNIT
A_XP = A_WO + 4 * 2048
XP_ROWS = XP * N2 + 24
A_Y = A_XP + 4 * XP_ROWS
A_F = A_Y + 2 * N1 * 2 * N2
A_ROWS = A_F + 2 * S + 8 * WP


def _pack_bf16(a):
    u = np.ascontiguousarray(a, dtype=np.float32).view(np.uint32)
    b = ((u + 0x7FFF + ((u >> 16) & 1)) >> 16).astype(np.uint32)
    return b[..., 0::2, :] | (b[..., 1::2, :] << 16)


def _dft_constants():
    lane = np.arange(128)
    k_even, k_odd = 2 * lane, 2 * lane + 1
    lo = lane % 2 == 0
    src = (lane - 1) % 128
    th = lambda n, k: 2 * np.pi * np.outer(n, k) / D
    fa = np.where(lo[None, :], np.cos(th(lane, k_even)), -np.sin(th(lane, k_even[src])))
    fa[:, 1] = np.cos(np.pi * lane)
    fb = np.where(~lo[None, :], np.cos(th(lane, k_even)), -np.sin(th(lane, k_even[src])))
    n = np.arange(256)
    fv = np.concatenate([np.cos(th(n, k_odd)), -np.sin(th(n, k_odd))], axis=1)
    sc = 1.0 / (S * D)
    wa = np.full(128, 2.0)
    wa[0] = wa[1] = 1.0
    ia, ib, iv = (fa * wa[None, :]).T * sc, fb.T * 2.0 * sc, fv.T * 2.0 * sc
    a32 = 2 * np.pi * np.outer(np.arange(N1), np.arange(N1)) / N1
    c32, s32 = np.zeros((128, 128)), np.zeros((128, 128))
    c32[:N1, :N1], s32[:N1, :N1] = np.cos(a32), np.sin(a32)
    cd = np.concatenate([fa, fb, fv[:, :128], fv[:, 128:], ia, ib, iv[:, :128], iv[:, 128:], c32, s32], axis=0)
    k2 = np.arange(N2)
    g = np.zeros((N1, 128, 128))
    for n1 in range(N1):
        ang = 2 * np.pi * np.outer(k2, n1 + N1 * k2) / S
        c, s = np.cos(ang), np.sin(ang)
        g[n1] = np.block([[c, s], [-s, c]])
    ang = 2 * np.pi * np.outer(k2, np.arange(N1)) / S
    tw = np.zeros((2, N2, 128), np.float32)
    tw[0, :, :N1], tw[1, :, :N1] = np.cos(ang), np.sin(ang)
    return _pack_bf16(cd), _pack_bf16(g), _pack_bf16(g.transpose(0, 2, 1)), tw


_CD, _G, _GT, _TW = _dft_constants()
_FA, _FB, _FVR, _FVI, _IA, _IB, _IV0, _IV1, _C32, _S32 = 0, 64, 128, 256, 384, 448, 512, 640, 768, 832


def _dot(a, b):
    return jnp.dot(a, b, preferred_element_type=F32)


def _as_bf16(u):
    return pltpu.bitcast(u, BF16)


def _cadd(a, b):
    return a[0] + b[0], a[1] + b[1]


def _csub(a, b):
    return a[0] - b[0], a[1] - b[1]


def _add_i(a, b):
    return a[0] - b[1], a[1] + b[0]


def _sub_i(a, b):
    return a[0] + b[1], a[1] - b[0]


def _twiddle(a, e, n):
    e %= n
    if e == 0:
        return a
    if 4 * e == n:
        return a[1], -a[0]
    if 4 * e == 3 * n:
        return -a[1], a[0]
    if 2 * e == n:
        return -a[0], -a[1]
    c, s = float(np.cos(2 * np.pi * e / n)), float(np.sin(2 * np.pi * e / n))
    if (8 * e) % n == 0:
        h = abs(c)
        if c > 0 and s > 0:
            return (a[0] + a[1]) * h, (a[1] - a[0]) * h
        if c < 0 and s > 0:
            return (a[1] - a[0]) * h, (a[0] + a[1]) * (-h)
        if c < 0 and s < 0:
            return (a[0] + a[1]) * (-h), (a[0] - a[1]) * h
        return (a[0] - a[1]) * h, (a[0] + a[1]) * h
    return a[0] * c + a[1] * s, a[1] * c - a[0] * s


def _radix4(z, sign):
    a, b, c, d = _cadd(z[0], z[2]), _csub(z[0], z[2]), _cadd(z[1], z[3]), _csub(z[1], z[3])
    if sign > 0:
        return [_cadd(a, c), _sub_i(b, d), _csub(a, c), _add_i(b, d)]
    return [_cadd(a, c), _add_i(b, d), _csub(a, c), _sub_i(b, d)]


def _fft8_fwd(z):
    ev = _radix4([_cadd(z[j], z[j + 4]) for j in range(4)], +1)
    d = [_csub(z[j], z[j + 4]) for j in range(4)]
    d1, d3 = _twiddle(d[1], 1, 8), _twiddle(d[3], 3, 8)
    a, b, c, e = _sub_i(d[0], d[2]), _add_i(d[0], d[2]), _cadd(d1, d3), _csub(d1, d3)
    od = [_cadd(a, c), _sub_i(b, e), _csub(a, c), _add_i(b, e)]
    return [ev[m // 2] if m % 2 == 0 else od[m // 2] for m in range(8)]


def _fft8_inv(x):
    ev = _radix4([x[0], x[2], x[4], x[6]], -1)
    od = _radix4([x[1], x[3], x[5], x[7]], -1)
    o1, o3 = _twiddle(od[1], -1, 8), _twiddle(od[3], -3, 8)
    lo = [_cadd(ev[0], od[0]), _cadd(ev[1], o1), _add_i(ev[2], od[2]), _cadd(ev[3], o3)]
    hi = [_csub(ev[0], od[0]), _csub(ev[1], o1), _sub_i(ev[2], od[2]), _csub(ev[3], o3)]
    return lo + hi


def _kernel(zero_ref, ax_hbm, wr_hbm, wi_hbm, bx_hbm, mem_hbm, wq_hbm, wk_hbm, wv_hbm, wo_hbm,
            cd_hbm, g_hbm, gt_hbm, tw_hbm, out_hbm,
            ax_v, wr_v, wi_v, bx_v, mem_v, wst, wo_st, cd_v, g_v, gt_v, tw_v,
            arena, x0_v, e_v, y0_v, b2_v, yn_v, yp, out_v,
            ring0, ring1, ring2, ring3, mq0, mq1, mq2, mq3,
            s0, s1, s2, s3, p0, p1, p2, p3, o0, o1, o2, o3,
            sems, out_sems, *, unroll, s_lag, a_lag, a_last, sm_start, sm_gap):
    rings, mems = (ring0, ring1, ring2, ring3), (mq0, mq1, mq2, mq3)
    s_scr, p_scr, o_scr = (s0, s1, s2, s3), (p0, p1, p2, p3), (o0, o1, o2, o3)
    w_hbm = (wq_hbm, wk_hbm, wv_hbm)
    P = functools.partial
    pin = pl.multiple_of(zero_ref[0], 8)

    copies = {}

    def add_copy(name, src, dst):
        copies[name] = pltpu.make_async_copy(src, dst, sems.at[len(copies)])

    for u in range(12):
        add_copy(u, w_hbm[u // 4].at[:, pl.ds(8 * (u % 4), 8), :], wst.at[u])
    add_copy("bx0", bx_hbm.at[pl.ds(0, R0)], bx_v.at[pl.ds(0, R0)])
    add_copy("bx1", bx_hbm.at[pl.ds(R0, S - R0)], bx_v.at[pl.ds(R0, S - R0)])
    add_copy("ax", ax_hbm, ax_v)
    add_copy("wr", wr_hbm, wr_v)
    add_copy("wi", wi_hbm, wi_v)
    add_copy("mem", mem_hbm, mem_v)
    add_copy("wo", wo_hbm, wo_st)
    add_copy("cd", cd_hbm, cd_v)
    add_copy("g", g_hbm, g_v)
    add_copy("gt", gt_hbm, gt_v)
    add_copy("tw", tw_hbm, tw_v)

    def sync(done, fresh):
        for n in done:
            copies[n].wait()
        for n in fresh:
            copies[n].start()

    lane = lax.broadcasted_iota(jnp.int32, (N2, 128), 1)
    lane2 = lax.broadcasted_iota(jnp.int32, (2 * N2, 128), 1)

    def cmat(off, rows):
        return _as_bf16(cd_v[off:off + rows // 2, :])

    def low(u):
        return pltpu.bitcast(u << 16, F32)

    def high(u):
        return pltpu.bitcast(u & jnp.uint32(0xFFFF0000), F32)

    def weight(w, hd, lo=0, hi=D // 2):
        base = A_WQKV + (4 * w + hd // 8) * UNIT + WP * (hd % 8)
        return _as_bf16(arena[base + lo:base + hi, :])

    def stage_piece(u, piece):
        sub = lax.broadcasted_iota(jnp.int32, (8, 128), 0)
        keep = jnp.where(sub < 4, jnp.uint32(0xFFFF), jnp.uint32(0xFFFF0000))
        words = pltpu.bitcast(wst[u, 32 * piece:32 * piece + 32].reshape(32 * 8, DH), U32)
        for j in range(16):
            v = words[8 * j:8 * j + 8]
            r = pltpu.roll(v, 4, 0)
            arena[pl.ds(pin + A_WQKV + u * UNIT + 16 * piece + j, 8, stride=WP), :] = (
                (v & keep) | (((r << 16) | (r >> 16)) & ~keep))

    def slot(hd):
        return hd - hd % 8 + (hd % 8) // 2 + 4 * (hd % 2)

    def project(u, hh, c):
        w, g = divmod(u, 4)
        lhs = jnp.concatenate([_as_bf16(x0_v[k, 64 * c:64 * c + 64, :]) for k in range(4)], axis=1)
        rings[g][8 * w + hh, pl.ds(RING - R0 + 128 * c, 128), :] = _dot(lhs, weight(w, slot(8 * g + hh)))

    def wo_relayout(n, c):
        arena[pl.ds(pin + A_WO + 2048 * n + 128 * c, 128), :] = pltpu.bitcast(
            wo_st[256 * c:256 * c + 256, 128 * n:128 * n + 128], U32)

    def a_decimate(n2):
        for c in range(4):
            arena[pl.ds(pin + A_XP + c * XP_ROWS + XP * n2, 16), :] = pltpu.bitcast(
                ax_v[32 * n2:32 * n2 + 32, 128 * c:128 * c + 128], U32)

    def a_fwd_d(a):
        xs = []
        for c in range(4):
            u = arena[pl.ds(A_XP + c * XP_ROWS + a, N2, stride=XP), :]
            xs.append(jnp.concatenate([low(u), high(u)], axis=0))
        u0, u1, v0, v1 = xs[0] + xs[2], xs[1] + xs[3], xs[0] - xs[2], xs[1] - xs[3]
        v = jnp.concatenate([v0, v1], axis=1)
        e_v[a % 2, 0] = _dot(u0 + u1, cmat(_FA, 128))
        e_v[a % 2, 1] = _dot(u0 - u1, cmat(_FB, 128))
        e_v[a % 2, 2] = _dot(v, cmat(_FVR, 256))
        e_v[a % 2, 3] = _dot(v, cmat(_FVI, 256))

    def a_fwd_s(a, p):
        n1 = 2 * a + p
        ea, eb, ore, oim = [e_v[a % 2, q, N2 * p:N2 * p + N2, :] for q in range(4)]
        even = (lane & 1) == 0
        ere = jnp.where(even, ea, eb)
        eim = pltpu.roll(jnp.where(even, eb, jnp.where(lane == 1, 0.0, ea)), 127, 1)
        nyq = pltpu.roll(ea, (n1 - 1) % 128, 1) if n1 != 1 else ea
        b2_v[...] = jnp.where(lane == n1, nyq, 0.0 if n1 == 0 else b2_v[...])
        gm = _as_bf16(g_v[n1])
        y0_v[0, n1] = _dot(gm, jnp.concatenate([ere, eim], axis=0).astype(BF16))
        y0_v[1, n1] = _dot(gm, jnp.concatenate([ore, oim], axis=0).astype(BF16))

    def filter_transpose(q, c):
        ref = (wr_v, wi_v)[q]
        arena[pl.ds(pin + A_F + S * q + 128 * c, 128), :] = pltpu.bitcast(ref[0:256, 128 * c:128 * c + 128], U32).T

    def yrow(t, n):
        return A_Y + (t * N1 + n) * 2 * N2

    def yget(t, n, j):
        row = yrow(t, n) + 8 * j
        return pltpu.bitcast(arena[row:row + 8, :], F32), pltpu.bitcast(arena[row + N2:row + N2 + 8, :], F32)

    def yput(t, n, j, z):
        row = yrow(t, n) + 8 * j
        arena[pl.ds(pin + row, 8), :] = pltpu.bitcast(z[0], U32)
        arena[pl.ds(pin + row + N2, 8), :] = pltpu.bitcast(z[1], U32)

    def fft_p1(t, j, j1):
        z = [(y0_v[t, j1 + 8 * q, 8 * j:8 * j + 8, :], y0_v[t, j1 + 8 * q, N2 + 8 * j:N2 + 8 * j + 8, :])
             for q in range(4)]
        o = _radix4(z, +1)
        for r in range(4):
            yput(t, 8 * r + j1, j, _twiddle(o[r], r * j1, N1))

    def fft_p2(t, j, r):
        x = _fft8_fwd([yget(t, 8 * r + j1, j) for j1 in range(8)])
        for m in range(8):
            row = N2 * (4 * m + r) + 8 * j
            fr, fi = [(low, high)[t](arena[A_F + S * q + row:A_F + S * q + row + 8, :]) for q in range(2)]
            x[m] = (x[m][0] * fr - x[m][1] * fi, x[m][0] * fi + x[m][1] * fr)
        z = _fft8_inv(x)
        for j1 in range(8):
            yput(t, 8 * r + j1, j, z[j1])

    def fft_p3(t, j, j1):
        z = _radix4([_twiddle(yget(t, 8 * r + j1, j), -r * j1, N1) for r in range(4)], -1)
        for q in range(4):
            yput(t, j1 + 8 * q, j, z[q])

    nyq = {}

    def nyq_1():
        rhs = jnp.concatenate([b2_v[...], jnp.zeros((N2, 128), F32)], axis=0).astype(BF16)
        nyq[1] = _dot(_as_bf16(g_v[0]), rhs)

    def nyq_2():
        y = nyq.pop(1)
        c, s = tw_v[0], tw_v[1]
        y = jnp.concatenate([y[:N2] * c + y[N2:] * s, y[N2:] * c - y[:N2] * s], axis=0)
        nyq[2] = _dot(y, cmat(_C32, 128)), _dot(y, cmat(_S32, 128))

    def nyq_filter(ref):
        row = lax.broadcasted_iota(jnp.int32, (N1, 128), 0)
        f = jnp.zeros((N1, 128), F32)
        for c in range(16):
            v = jnp.broadcast_to(ref[256:257, 128 * c:128 * c + 128].astype(F32), (8, 128))
            f = jnp.where(row == 2 * c, jnp.concatenate([v] * 4, axis=0), f)
            f = jnp.where(row == 2 * c + 1, jnp.concatenate([pltpu.roll(v, 64, 1)] * 4, axis=0), f)
        return jnp.concatenate([f, jnp.zeros((128 - N1, 128), F32)], axis=0).T[:N2]

    def nyq_3():
        yc, ys = nyq.pop(2)
        xr, xi = yc[:N2] + ys[N2:], yc[N2:] - ys[:N2]
        fr, fi = nyq_filter(wr_v), nyq_filter(wi_v)
        x = jnp.concatenate([xr * fr - xi * fi, xr * fi + xi * fr], axis=0)
        nyq[3] = _dot(x, cmat(_C32, 128)), _dot(x, cmat(_S32, 128))

    def nyq_4():
        xc, xs = nyq.pop(3)
        tr, ti = xc[:N2] - xs[N2:], xc[N2:] + xs[:N2]
        c, s = tw_v[0], tw_v[1]
        t = jnp.concatenate([tr * c - ti * s, ti * c + tr * s], axis=0).astype(BF16)
        yn_v[...] = _dot(_as_bf16(gt_v[0, 0:N2 // 2, :]), t)

    def a_inv_s(a, p):
        gm = _as_bf16(gt_v[2 * a + p])
        for t in range(2):
            row = yrow(t, 2 * a + p)
            r = _dot(gm, pltpu.bitcast(arena[row:row + 2 * N2, :], F32).astype(BF16))
            e_v[a % 2, 2 * t, N2 * p:N2 * p + N2, :] = r[:N2]
            e_v[a % 2, 2 * t + 1, N2 * p:N2 * p + N2, :] = r[N2:]

    def a_inv_d(a):
        even = (lane2 & 1) == 0
        ere, eim = e_v[a % 2, 0], pltpu.roll(e_v[a % 2, 1], 1, 1)
        yn = yn_v[...]
        nq = jnp.concatenate([pltpu.roll(yn, (1 - n1) % 128, 1) if n1 != 1 else yn
                              for n1 in (2 * a, 2 * a + 1)], axis=0)
        ea = _dot(jnp.where(lane2 == 1, nq, jnp.where(even, ere, eim)), cmat(_IA, 128))
        eb = _dot(jnp.where(even, eim, ere), cmat(_IB, 128))
        o = jnp.concatenate([e_v[a % 2, 2], e_v[a % 2, 3]], axis=1)
        v0, v1 = _dot(o, cmat(_IV0, 256)), _dot(o, cmat(_IV1, 256))
        pp, qq = ea + eb, ea - eb
        for c, y in enumerate((pp + v0, qq + v1, pp - v0, qq - v1)):
            for p in range(2):
                yp[c, pl.ds(2 * a + p, N2, stride=YP), :] = y[N2 * p:N2 * p + N2]

    main = [P(project, u, hh, c) for u in range(12) for hh in range(8) for c in range(4)]
    side = {}

    def spread(tasks, lo, hi):
        for j, f in enumerate(tasks):
            side.setdefault(lo + (j * (hi - lo)) // len(tasks), []).append(f)

    syncs = {16: ([1], [3, "ax"]), 34: ([2], ["g", "cd", 4]), 66: ([3, "ax"], [5, 6, 7]),
             98: ([4, "g", "cd"], ["wr", "wi", "tw", 8]), 130: ([5, 6, 7, "wr", "wi", "tw"], [9, "gt", 10, 11]),
             226: ([8, 9, "gt"], ["wo", "bx1", "mem"]), 290: ([10, 11, "wo", "bx1", "mem"], [])}
    for pos, (done, fresh) in syncs.items():
        spread([P(sync, done, fresh)], pos, pos + 1)
    for u in range(1, 12):
        spread([P(stage_piece, u, piece) for piece in range(16)], 32 * u - (16 if u == 1 else 30), 32 * u - 2)
    spread([P(a_decimate, n2) for n2 in range(N2)], 66, 98)
    tasks = [P(a_fwd_d, 0)]
    for a in range(16):
        tasks += ([P(a_fwd_d, a + 1)] if a + 1 < 16 else []) + [P(a_fwd_s, a, 0), P(a_fwd_s, a, 1)]
    spread(tasks, 98, 162)
    groups = [(t, j) for j in range(8) for t in range(2)]
    spread([P(filter_transpose, q, c) for c in range(16) for q in range(2)], 130, 194)
    spread([P(fft_p1, t, j, j1) for t, j in groups for j1 in range(8)], 164, 196)
    spread([P(fft_p2, t, j, r) for t, j in groups for r in range(4)], 196, 290)
    spread([P(fft_p3, t, j, j1) for t, j in groups for j1 in range(8)], 290, 322)
    spread([nyq_1, nyq_2, nyq_3], 166, 178)
    spread([nyq_4], 230, 231)
    spread([P(wo_relayout, n, c) for c in range(16) for n in range(4)], 320, 382)
    tasks = [P(a_inv_s, 0, 0), P(a_inv_s, 0, 1)]
    for a in range(16):
        tasks += ([P(a_inv_s, a + 1, 0), P(a_inv_s, a + 1, 1)] if a + 1 < 16 else []) + [P(a_inv_d, a)]
    spread(tasks, 323, 383)

    sync([], ["bx0", 0])
    sync(["bx0"], [])
    for k in range(4):
        x0_v[k] = pltpu.bitcast(bx_v[0:R0, 128 * k:128 * k + 128], U32)
    sync([0], [1, 2])
    for piece in range(16):
        stage_piece(0, piece)
    for i, f in enumerate(main):
        for e in side.get(i, []):
            e()
        f()

    scale = DH ** -0.5 * LOG2E

    def step(s, m):
        rows = lax.broadcasted_iota(jnp.int32, (2 * L, 128), 0)
        cols = lax.broadcasted_iota(jnp.int32, (2 * L, 128), 1)
        rl = jnp.where(rows >= L, rows - L, rows)
        cl = jnp.where(cols >= L, cols - L, cols)
        same = ((rows >= L) == (cols >= L)) & (cols < 2 * L)
        valid = same & ((rl < M) | (rl >= cl))
        fill = jnp.where(same, -1e9 * LOG2E, -jnp.inf).astype(F32)
        xs = bx_v[pl.ds(pl.multiple_of(R0 + s * RX, 8), RX), :].astype(F32)
        wpos = pl.multiple_of(lax.rem(s * RX, RING), 8)
        rpos = pl.multiple_of(lax.rem(RING - R0 + s * SEG, RING), SEG)
        hk = [jnp.concatenate([xs[:, 128 * k:128 * (k + 1)], m[k]], axis=0) for k in range(4)]
        h4 = jnp.concatenate(hk, axis=1)
        h3 = jnp.concatenate(hk[:3], axis=1)

        def put(w, hd, y):
            g, i = divmod(hd, 8)
            mems[g][8 * w + i] = y[RX:]
            rings[g][8 * w + i, pl.ds(wpos, RX), :] = y[:RX]

        def get(w, hd):
            g, i = divmod(hd, 8)
            return [mems[g][8 * w + i], rings[g][8 * w + i, pl.ds(rpos, SEG), :]]

        def proj(w, hd):
            put(w, hd, _dot(h4, weight(w, slot(hd))))

        part = {}

        def proj_a(w, hd):
            part[w, hd] = _dot(h3, weight(w, slot(hd), 0, 192))

        def proj_b(w, hd):
            put(w, hd, part.pop((w, hd)) + _dot(hk[3], weight(w, slot(hd), 192, 256)))

        def keys(w, j):
            kv = jnp.concatenate(get(w, 2 * j) + get(w, 2 * j + 1), axis=0).astype(BF16)
            return jnp.concatenate([kv, jnp.zeros((128 - 2 * L, DH), BF16)], axis=0)

        def scores(j):
            q2 = jnp.concatenate(get(0, 2 * j) + get(0, 2 * j + 1), axis=0)
            s_scr[j // 4][j % 4] = lax.dot_general(q2, keys(1, j), (((1,), (1,)), ((), ())),
                                                   preferred_element_type=F32)

        def softmax(j):
            sc = jnp.where(valid, s_scr[j // 4][j % 4] * scale, fill)
            e = jnp.exp2(sc - jnp.max(sc, axis=-1, keepdims=True))
            p_scr[j // 4][j % 4] = (e * (1.0 / jnp.sum(e, axis=-1, keepdims=True))).astype(BF16)

        def pv(j):
            o2 = _dot(p_scr[j // 4][j % 4], keys(2, j))
            o_scr[j // 4][2 * (j % 4)] = o2[:L]
            o_scr[j // 4][2 * (j % 4) + 1] = o2[L:]

        accs = [None] * 4

        def wo(g, n):
            lhs = jnp.concatenate([o_scr[g // 2][4 * (g % 2) + i] for i in range(4)], axis=1)
            row = A_WO + 2048 * n + 256 * g
            y = _dot(lhs, _as_bf16(arena[row:row + 256, :]))
            accs[n] = y if accs[n] is None else accs[n] + y

        order = [(w, hd) for hd in range(H) for w in (0, 1)] + [(2, hd) for hd in range(H)]

        def head():
            proj_a(*order[3])
            for t in order[:4]:
                proj_b(*t)

        main = [P(proj_a, *t) for t in order[:3]] + [head] + [P(proj, *t) for t in order[4:]]
        main += [P(wo, g, n) for g in range(8) for n in range(3)] + [P(wo, g, 3) for g in range(8)]
        extra = {}
        for g in range(4):
            pos = 16 * (g + 1) + s_lag
            for jj in range(4):
                extra.setdefault(pos, []).append(P(scores, 4 * g + jj))
            for jj in range(4):
                extra.setdefault(pos + sm_start + sm_gap * jj, []).append(P(softmax, 4 * g + jj))
            pos = 64 + 8 * (g + 1) + (a_lag if g < 3 else a_last)
            for jj in range(4):
                extra.setdefault(pos, []).append(P(pv, 4 * g + jj))
        for i, f in enumerate(main):
            for e in extra.get(i, []):
                e()
            f()
        rows = pl.ds(pl.multiple_of(s * SEG, SEG), SEG)
        for c in range(4):
            out_v[rows, 128 * c:128 * c + 128] = yp[c, pl.ds(s * YP, SEG), :].astype(BF16)
            out_v[rows, D + 128 * c:D + 128 * c + 128] = accs[c][M:].astype(BF16)
        return [a[:M] for a in accs]

    chunk = SEG * unroll

    def out_b_copy(i):
        rows = pl.ds(pl.multiple_of(i * chunk, chunk), chunk)
        return pltpu.make_async_copy(out_v.at[rows], out_hbm.at[rows], out_sems)

    def body(i, m):
        for u in range(unroll):
            m = step(i * unroll + u, m)
        out_b_copy(i).start()
        return m

    m0 = mem_v[...].astype(F32)
    lax.fori_loop(0, NSEG // unroll, body, [m0[:, 128 * k:128 * (k + 1)] for k in range(4)])

    def drain(i, c):
        out_b_copy(i).wait()
        return c

    lax.fori_loop(0, NSEG // unroll, drain, 0)


def make(unroll=2, s_lag=6, a_lag=6, a_last=5, sm_start=3, sm_gap=2, flags=None, interpret=False):
    vm = pltpu.VMEM
    scratch = [
        vm((S, D), BF16), vm((D // 2 + 1, S), BF16), vm((D // 2 + 1, S), BF16), vm((S, D), BF16), vm((M, D), BF16),
        vm((12, D, 8, DH), BF16), vm((H * DH, D), BF16),
        vm(_CD.shape, U32), vm(_G.shape, U32), vm(_GT.shape, U32), vm(_TW.shape, F32),
        vm((A_ROWS, 128), U32), vm((4, R0 // 2, 128), U32), vm((2, 4, 2 * N2, 128), F32),
        vm((2, N1, 2 * N2, 128), F32), vm((N2, 128), F32), vm((N2, 128), F32), vm((4, YP * N2 + 40, 128), F32),
        vm((S, 2 * D), BF16),
    ]
    scratch += [vm((24, RING, DH), F32)] * 4 + [vm((24, M, DH), F32)] * 4
    scratch += [vm((4, 2 * L, 128), F32)] * 4 + [vm((4, 2 * L, 128), BF16)] * 4 + [vm((8, L, DH), F32)] * 4
    scratch += [pltpu.SemaphoreType.DMA((23,)), pltpu.SemaphoreType.DMA(())]
    kern = functools.partial(_kernel, unroll=unroll, s_lag=s_lag, a_lag=a_lag, a_last=a_last,
                             sm_start=sm_start, sm_gap=sm_gap)

    @jax.jit
    def f(A_x, A_w_r, A_w_i, B_x, B_mem0, B_Wq, B_Wk, B_Wv, B_Wo):
        out = pl.pallas_call(
            kern,
            out_shape=jax.ShapeDtypeStruct((S, 2 * D), BF16),
            in_specs=[pl.BlockSpec(memory_space=pltpu.SMEM)] + [pl.BlockSpec(memory_space=pltpu.HBM)] * 13,
            out_specs=pl.BlockSpec(memory_space=pltpu.HBM),
            scratch_shapes=scratch,
            compiler_params=pltpu.CompilerParams(vmem_limit_bytes=120 * 1024 * 1024, flags=flags),
            interpret=interpret,
        )(np.zeros((1,), np.int32), A_x.reshape(S, D), A_w_r.T, A_w_i.T, B_x.reshape(S, D), B_mem0.reshape(M, D), B_Wq, B_Wk, B_Wv,
          B_Wo.reshape(H * DH, D), _CD, _G, _GT, _TW)
        return out.reshape(1, S, 2 * D)

    return f


_run = make(unroll=1)


def pallas_concat_heads__spectral_gfnet__memory_aug_recurrent_mem_tr__prompt_kernel(
        A_x, A_w_r, A_w_i, B_x, B_mem0, B_Wq, B_Wk, B_Wv, B_Wo, B_seg_len):
    assert int(B_seg_len) == SEG and A_x.shape == (1, S, D) and B_Wq.shape == (D, H, DH)
    return _run(A_x, A_w_r, A_w_i, B_x, B_mem0, B_Wq, B_Wk, B_Wv, B_Wo)
```

```python
import functools

import jax
import jax.numpy as jnp
import numpy as np
from jax import lax
from jax.experimental import pallas as pl
from jax.experimental.pallas import tpu as pltpu

F32, BF16, U32 = jnp.float32, jnp.bfloat16, jnp.uint32

S, D = 2048, 512
H, DH, M, SEG = 32, 128, 8, 32
L = M + SEG
NSEG = S // SEG
N1, N2 = 32, 64
R0, RX = 512, 24
RING = 576
XP, YP, TP = 17, 40, 9
LOG2E = 1.4426950408889634
UNIT = 8 * D // 2
TMP_ROWS = TP * (D // 2)
A_WQKV = 0
A_TMP = A_WQKV + 12 * UNIT
A_SUMS = A_TMP + 2 * TMP_ROWS + 16
A_XP = A_SUMS + 2 * 5 * 128
XP_ROWS = XP * N2 + 24
A_Y = A_XP + 4 * XP_ROWS
A_ROWS = A_Y + 2 * N1 * 2 * N2


def _pack_bf16(a):
    u = np.ascontiguousarray(a, dtype=np.float32).view(np.uint32)
    b = ((u + 0x7FFF + ((u >> 16) & 1)) >> 16).astype(np.uint32)
    return b[..., 0::2, :] | (b[..., 1::2, :] << 16)


def _dft_constants():
    lane = np.arange(128)
    k_even, k_odd = 2 * lane, 2 * lane + 1
    lo = lane % 2 == 0
    src = (lane - 1) % 128
    th = lambda n, k: 2 * np.pi * np.outer(n, k) / D
    fa = np.where(lo[None, :], np.cos(th(lane, k_even)), -np.sin(th(lane, k_even[src])))
    fa[:, 1] = np.cos(np.pi * lane)
    fb = np.where(~lo[None, :], np.cos(th(lane, k_even)), -np.sin(th(lane, k_even[src])))
    p, q = np.cos(th(lane, k_odd)), -np.sin(th(lane, k_odd))
    sign = np.where(lo, -1.0, 1.0)[None, :]
    f2, f3 = q - sign * p, p + sign * q
    sc = 1.0 / (S * D)
    wa = np.full(128, 2.0)
    wa[0] = wa[1] = 1.0
    ia, ib = (fa * wa[None, :]).T * sc, fb.T * 2.0 * sc
    i1, i2, i3 = p.T * 2.0 * sc, (sign * f2).T * 2.0 * sc, f3.T * 2.0 * sc
    a32 = 2 * np.pi * np.outer(np.arange(N1), np.arange(N1)) / N1
    c32, s32 = np.zeros((128, 128)), np.zeros((128, 128))
    c32[:N1, :N1], s32[:N1, :N1] = np.cos(a32), np.sin(a32)
    cd = np.concatenate([fa, fb, p, f2, f3, ia, ib, i1, i2, i3, c32, s32], axis=0)
    k2 = np.arange(N2)
    g = np.zeros((N1, 128, 128))
    for n1 in range(N1):
        ang = 2 * np.pi * np.outer(k2, n1 + N1 * k2) / S
        c, s = np.cos(ang), np.sin(ang)
        g[n1] = np.block([[c, s], [-s, c]])
    ang = 2 * np.pi * np.outer(k2, np.arange(N1)) / S
    tw = np.zeros((2, N2, 128), np.float32)
    tw[0, :, :N1], tw[1, :, :N1] = np.cos(ang), np.sin(ang)
    return _pack_bf16(cd), _pack_bf16(g), _pack_bf16(g.transpose(0, 2, 1)), tw


_CD, _G, _GT, _TW = _dft_constants()
_FA, _FB, _F1, _F2, _F3, _IA, _IB, _I1, _I2, _I3, _C32, _S32 = range(0, 12 * 64, 64)


def _dot(a, b):
    return jnp.dot(a, b, preferred_element_type=F32)


def _as_bf16(u):
    return pltpu.bitcast(u, BF16)


def _cadd(a, b):
    return a[0] + b[0], a[1] + b[1]


def _csub(a, b):
    return a[0] - b[0], a[1] - b[1]


def _add_i(a, b):
    return a[0] - b[1], a[1] + b[0]


def _sub_i(a, b):
    return a[0] + b[1], a[1] - b[0]


def _twiddle(a, e, n):
    e %= n
    if e == 0:
        return a
    if 4 * e == n:
        return a[1], -a[0]
    if 4 * e == 3 * n:
        return -a[1], a[0]
    if 2 * e == n:
        return -a[0], -a[1]
    c, s = float(np.cos(2 * np.pi * e / n)), float(np.sin(2 * np.pi * e / n))
    if (8 * e) % n == 0:
        h = abs(c)
        if c > 0 and s > 0:
            return (a[0] + a[1]) * h, (a[1] - a[0]) * h
        if c < 0 and s > 0:
            return (a[1] - a[0]) * h, (a[0] + a[1]) * (-h)
        if c < 0 and s < 0:
            return (a[0] + a[1]) * (-h), (a[0] - a[1]) * h
        return (a[0] - a[1]) * h, (a[0] + a[1]) * h
    return a[0] * c + a[1] * s, a[1] * c - a[0] * s


def _radix4(z, sign):
    a, b, c, d = _cadd(z[0], z[2]), _csub(z[0], z[2]), _cadd(z[1], z[3]), _csub(z[1], z[3])
    if sign > 0:
        return [_cadd(a, c), _sub_i(b, d), _csub(a, c), _add_i(b, d)]
    return [_cadd(a, c), _add_i(b, d), _csub(a, c), _sub_i(b, d)]


def _fft8_fwd(z):
    ev = _radix4([_cadd(z[j], z[j + 4]) for j in range(4)], +1)
    d = [_csub(z[j], z[j + 4]) for j in range(4)]
    d1, d3 = _twiddle(d[1], 1, 8), _twiddle(d[3], 3, 8)
    a, b, c, e = _sub_i(d[0], d[2]), _add_i(d[0], d[2]), _cadd(d1, d3), _csub(d1, d3)
    od = [_cadd(a, c), _sub_i(b, e), _csub(a, c), _add_i(b, e)]
    return [ev[m // 2] if m % 2 == 0 else od[m // 2] for m in range(8)]


def _fft8_inv(x):
    ev = _radix4([x[0], x[2], x[4], x[6]], -1)
    od = _radix4([x[1], x[3], x[5], x[7]], -1)
    o1, o3 = _twiddle(od[1], -1, 8), _twiddle(od[3], -3, 8)
    lo = [_cadd(ev[0], od[0]), _cadd(ev[1], o1), _add_i(ev[2], od[2]), _cadd(ev[3], o3)]
    hi = [_csub(ev[0], od[0]), _csub(ev[1], o1), _sub_i(ev[2], od[2]), _csub(ev[3], o3)]
    return lo + hi


def _kernel(zero_ref, ax_hbm, wr_hbm, wi_hbm, bx_hbm, mem_hbm, wq_hbm, wk_hbm, wv_hbm, wo_hbm,
            cd_hbm, g_hbm, gt_hbm, tw_hbm, out_hbm,
            ax_v, wr_v, wi_v, bx_v, mem_v, wst, wo_st, cd_v, g_v, gt_v, tw_v,
            arena, f_v, sum_v, tmp_v, x0_v, xq_v, e_v, y0_v, b2_v, yn_v, yp, out_v,
            ring0, ring1, ring2, ring3, mq0, mq1, mq2, mq3,
            s0, s1, s2, s3, p0, p1, p2, p3, o0, o1, o2, o3,
            sems, out_sems, *, unroll, s_lag, a_lag, a_last, sm_start, sm_gap, nseg, prologue, window, plan):
    rings, mems = (ring0, ring1, ring2, ring3), (mq0, mq1, mq2, mq3)
    s_scr, p_scr, o_scr = (s0, s1, s2, s3), (p0, p1, p2, p3), (o0, o1, o2, o3)
    w_hbm = (wq_hbm, wk_hbm, wv_hbm)
    P = functools.partial
    pin = pl.multiple_of(zero_ref[0], 8)

    copies = {}

    def add_copy(name, src, dst):
        copies[name] = pltpu.make_async_copy(src, dst, sems.at[len(copies)])

    for u in range(1, 12):
        add_copy(u, w_hbm[u // 4].at[:, pl.ds(8 * (u % 4), 8), :], wst.at[u])
    for q in range(4):
        add_copy(("w0", q), wq_hbm.at[pl.ds(128 * q, 128), pl.ds(0, 8), :], wst.at[0, pl.ds(128 * q, 128)])
    add_copy("bx0", bx_hbm.at[pl.ds(0, R0)], bx_v.at[pl.ds(0, R0)])
    add_copy("bx1", bx_hbm.at[pl.ds(R0, S - R0)], bx_v.at[pl.ds(R0, S - R0)])
    add_copy("ax", ax_hbm, ax_v)
    add_copy("wr", wr_hbm, wr_v)
    add_copy("wi", wi_hbm, wi_v)
    add_copy("mem", mem_hbm, mem_v)
    for n in range(4):
        add_copy(("wo", n), wo_hbm.at[:, pl.ds(128 * n, 128)], wo_st.at[n])
    add_copy("cd", cd_hbm, cd_v)
    add_copy("g", g_hbm, g_v)
    add_copy("gt", gt_hbm, gt_v)
    add_copy("tw", tw_hbm, tw_v)

    def sync(done, fresh):
        with jax.named_scope("sync_" + "_".join(str(n) for n in done)):
            for n in done:
                copies[n].wait()
            for n in fresh:
                copies[n].start()

    lane = lax.broadcasted_iota(jnp.int32, (N2, 128), 1)
    lane2 = lax.broadcasted_iota(jnp.int32, (2 * N2, 128), 1)
    lane_sign = jnp.where((lane2 & 1) == 0, -1.0, 1.0).astype(F32)

    def cmat(off, rows):
        return _as_bf16(cd_v[off:off + rows // 2, :])

    def low(u):
        return pltpu.bitcast(u << 16, F32)

    def high(u):
        return pltpu.bitcast(u & jnp.uint32(0xFFFF0000), F32)

    tmp_ref, tmp_off = (arena, A_TMP) if plan.get("tmp_arena", True) else (tmp_v, 0)
    sum_ref, sum_off = (arena, A_SUMS) if plan.get("sum_arena", True) else (sum_v, 0)

    def tile_row(u, i):
        return A_WQKV + u * UNIT + (D // 2) * i

    def weight(w, hd, lo=0, hi=D // 2):
        base = tile_row(4 * w + hd // 8, hd % 8)
        return _as_bf16(arena[base + lo:base + hi, :])

    def stage_piece(u, piece):
        words = pltpu.bitcast(wst[u, 32 * piece:32 * piece + 32].reshape(32 * 8, DH), U32)
        yield
        for j in range(16):
            row = (u % 2) * TMP_ROWS + TP * (16 * piece + j)
            tmp_ref[pl.ds(pin + tmp_off + row, 8), :] = words[8 * j:8 * j + 8]

    def relayout(pair, k, sums):
        u, i = divmod(pair, 4)
        halves = [[tmp_ref[pl.ds(tmp_off + (u % 2) * TMP_ROWS + TP * (128 * half + 16 * k) + i + 4 * q, 16, stride=TP), :]
                   for q in range(2)] for half in range(2)]
        yield
        for half, (ev, od) in enumerate(halves):
            row = (0 if sums else pin) + tile_row(u, 2 * i) + 128 * half + 16 * k
            arena[pl.ds(row, 16), :] = (ev & jnp.uint32(0xFFFF)) | (od << 16)
            arena[pl.ds(row + D // 2, 16), :] = (ev >> 16) | (od & jnp.uint32(0xFFFF0000))
        if sums:
            b11, b12, b21, b22 = [(f(ev), f(od)) for ev, od in halves for f in (low, high)]
            for n, t in enumerate((_cadd(b11, b22), _csub(b12, b22), _csub(b21, b11), _cadd(b11, b12),
                                   _cadd(b21, b22))):
                ev, od = [pltpu.bitcast(v, U32) + jnp.uint32(0x8000) for v in t]
                sum_ref[pl.ds(pin + sum_off + ((pair % 2) * 5 + n) * 128 + 16 * k, 16), :] = (
                    (ev >> 16) | (od & jnp.uint32(0xFFFF0000)))

    def project_big(pair, c, part):
        w, g = divmod(pair // 4, 4)
        row = tile_row(pair // 4, 2 * (pair % 4))

        def product(i):
            lhs = jnp.concatenate([_as_bf16(x0_v[i - 1, k, 64 * c:64 * c + 64, :]) for k in range(2)], axis=1)
            if i == 2:
                rhs = arena[row:row + 128, :]
            elif i == 5:
                rhs = arena[row + D // 2 + 128:row + D // 2 + 256, :]
            else:
                r0 = sum_off + ((pair % 2) * 5 + (1, 3, 4, 6, 7).index(i)) * 128
                rhs = sum_ref[r0:r0 + 128, :]
            return _dot(lhs, _as_bf16(rhs))

        def put(r, n, y):
            rings[g][8 * w + 2 * (pair % 4) + n, pl.ds(RING - R0 + 256 * r + 128 * c, 128), :] = y

        if part == 0:
            m3, m5 = product(3), product(5)
            put(0, 1, m3 + m5)
            carry[0] = (m5, m3)
        elif part == 1:
            m5, m3 = carry.pop(0)
            m2, m4 = product(2), product(4)
            put(1, 0, m2 + m4)
            carry[0] = (m4 - m5, m3 - m2)
        elif part == 2:
            t11, t22 = carry.pop(0)
            m1, m7 = product(1), product(7)
            put(0, 0, m1 + m7 + t11)
            carry[0] = m1 + t22
        else:
            put(1, 1, product(6) + carry.pop(0))

    def project_plain(pair, n, c):
        w, g = divmod(pair // 4, 4)
        hh = 2 * (pair % 4) + n
        lhs = jnp.concatenate([_as_bf16(xq_v[k, 64 * c:64 * c + 64, :]) for k in range(4)], axis=1)
        rings[g][8 * w + hh, pl.ds(RING - R0 + 128 * c, 128), :] = _dot(lhs, weight(w, 8 * g + hh))

    def token_sums():
        def quad(r, k):
            return bx_v[256 * r:256 * r + 256, 256 * k:256 * k + 256].astype(F32)

        for k in range(4):
            xq_v[k] = pltpu.bitcast(bx_v[0:R0, 128 * k:128 * k + 128], U32)
        a11, a12, a21, a22 = quad(0, 0), quad(0, 1), quad(1, 0), quad(1, 1)
        for i, t in enumerate((a11 + a22, a21 + a22, a11, a22, a11 + a12, a21 - a11, a12 - a22)):
            for k in range(2):
                x0_v[i, k] = pltpu.bitcast(t[:, 128 * k:128 * k + 128].astype(BF16), U32)

    carry = {}

    def project(pair, c, half):
        w, g = divmod(pair // 4, 4)
        row = tile_row(pair // 4, 2 * (pair % 4))

        def product(i):
            lhs = jnp.concatenate([_as_bf16(x0_v[i - 1, k, 32 * c:32 * c + 32, :]) for k in range(2)], axis=1)
            if i == 2:
                rhs = arena[row:row + 128, :]
            elif i == 5:
                rhs = arena[row + D // 2 + 128:row + D // 2 + 256, :]
            else:
                r0 = sum_off + ((pair % 2) * 5 + (1, 3, 4, 6, 7).index(i)) * 128
                rhs = sum_ref[r0:r0 + 128, :]
            return _dot(lhs, _as_bf16(rhs))

        def put(r, n, y):
            rings[g][8 * w + 2 * (pair % 4) + n, pl.ds(RING - R0 + 256 * r + 64 * c, 64), :] = y

        if half == 0:
            m3, m5, m2, m4 = product(3), product(5), product(2), product(4)
            put(0, 1, m3 + m5)
            put(1, 0, m2 + m4)
            carry[0] = (m4 - m5, m3 - m2)
        else:
            t11, t22 = carry.pop(0)
            m1, m7, m6 = product(1), product(7), product(6)
            put(0, 0, m1 + m7 + t11)
            put(1, 1, m1 + m6 + t22)

    def a_decimate(n2):
        yield
        for c in range(4):
            arena[pl.ds(pin + A_XP + c * XP_ROWS + XP * n2, 16), :] = pltpu.bitcast(
                ax_v[32 * n2:32 * n2 + 32, 128 * c:128 * c + 128], U32)

    def a_fwd_d(a):
        xs = []
        for c in range(4):
            u = arena[pl.ds(A_XP + c * XP_ROWS + a, N2, stride=XP), :]
            xs.append(jnp.concatenate([low(u), high(u)], axis=0))
        u0, u1, v0, v1 = xs[0] + xs[2], xs[1] + xs[3], xs[0] - xs[2], xs[1] - xs[3]
        e_v[a % 2, 0] = _dot(u0 + u1, cmat(_FA, 128))
        e_v[a % 2, 1] = _dot(u0 - u1, cmat(_FB, 128))
        k1 = _dot(v0 + v1, cmat(_F1, 128))
        e_v[a % 2, 2] = k1 - _dot(v1, cmat(_F3, 128))
        e_v[a % 2, 3] = k1 * lane_sign + _dot(v0, cmat(_F2, 128))

    def a_fwd_s(a, p):
        n1 = 2 * a + p
        ea, eb, ore, oim = [e_v[a % 2, q, N2 * p:N2 * p + N2, :] for q in range(4)]
        even = (lane & 1) == 0
        ere = jnp.where(even, ea, eb)
        eim = pltpu.roll(jnp.where(even, eb, jnp.where(lane == 1, 0.0, ea)), 127, 1)
        nyq = pltpu.roll(ea, (n1 - 1) % 128, 1) if n1 != 1 else ea
        b2_v[...] = jnp.where(lane == n1, nyq, 0.0 if n1 == 0 else b2_v[...])
        gm = _as_bf16(g_v[n1])
        y0_v[0, n1] = _dot(gm, jnp.concatenate([ere, eim], axis=0).astype(BF16))
        y0_v[1, n1] = _dot(gm, jnp.concatenate([ore, oim], axis=0).astype(BF16))

    def filter_transpose(q, c):
        ref = (wr_v, wi_v)[q]
        f_v[q, 128 * c:128 * c + 128, :] = pltpu.bitcast(ref[0:256, 128 * c:128 * c + 128], U32).T

    def yrow(t, n):
        return A_Y + (t * N1 + n) * 2 * N2

    def yget(t, n, j):
        row = yrow(t, n) + 8 * j
        return pltpu.bitcast(arena[row:row + 8, :], F32), pltpu.bitcast(arena[row + N2:row + N2 + 8, :], F32)

    def yput(t, n, j, z):
        row = yrow(t, n) + 8 * j
        arena[pl.ds(pin + row, 8), :] = pltpu.bitcast(z[0], U32)
        arena[pl.ds(pin + row + N2, 8), :] = pltpu.bitcast(z[1], U32)

    def fft_p1(t, j, j1):
        z = [(y0_v[t, j1 + 8 * q, 8 * j:8 * j + 8, :], y0_v[t, j1 + 8 * q, N2 + 8 * j:N2 + 8 * j + 8, :])
             for q in range(4)]
        o = _radix4(z, +1)
        yield
        for r in range(4):
            yput(t, 8 * r + j1, j, _twiddle(o[r], r * j1, N1))

    def fft_p2(t, j, r):
        x = _fft8_fwd([yget(t, 8 * r + j1, j) for j1 in range(8)])
        for m in range(8):
            row = N2 * (4 * m + r) + 8 * j
            fr, fi = [(low, high)[t](f_v[q, row:row + 8, :]) for q in range(2)]
            x[m] = (x[m][0] * fr - x[m][1] * fi, x[m][0] * fi + x[m][1] * fr)
        z = _fft8_inv(x)
        yield
        for j1 in range(8):
            yput(t, 8 * r + j1, j, z[j1])

    def fft_p3(t, j, half):
        cols = range(4 * half, 4 * half + 4)
        o = {j1: [yget(t, 8 * r + j1, j) for r in range(4)] for j1 in cols}
        yield
        for j1 in cols:
            z = _radix4([_twiddle(o[j1][r], -r * j1, N1) for r in range(4)], -1)
            for q in range(4):
                yput(t, j1 + 8 * q, j, z[q])

    nyq = {}

    def nyq_1():
        rhs = jnp.concatenate([b2_v[...], jnp.zeros((N2, 128), F32)], axis=0).astype(BF16)
        nyq[1] = _dot(_as_bf16(g_v[0]), rhs)

    def nyq_2():
        y = nyq.pop(1)
        c, s = tw_v[0], tw_v[1]
        y = jnp.concatenate([y[:N2] * c + y[N2:] * s, y[N2:] * c - y[:N2] * s], axis=0)
        nyq[2] = _dot(y, cmat(_C32, 128)), _dot(y, cmat(_S32, 128))

    def nyq_filter(ref):
        row = lax.broadcasted_iota(jnp.int32, (N1, 128), 0)
        f = jnp.zeros((N1, 128), F32)
        for c in range(16):
            v = jnp.broadcast_to(ref[256:257, 128 * c:128 * c + 128].astype(F32), (8, 128))
            f = jnp.where(row == 2 * c, jnp.concatenate([v] * 4, axis=0), f)
            f = jnp.where(row == 2 * c + 1, jnp.concatenate([pltpu.roll(v, 64, 1)] * 4, axis=0), f)
        return jnp.concatenate([f, jnp.zeros((128 - N1, 128), F32)], axis=0).T[:N2]

    def nyq_3():
        yc, ys = nyq.pop(2)
        xr, xi = yc[:N2] + ys[N2:], yc[N2:] - ys[:N2]
        fr, fi = nyq_filter(wr_v), nyq_filter(wi_v)
        x = jnp.concatenate([xr * fr - xi * fi, xr * fi + xi * fr], axis=0)
        nyq[3] = _dot(x, cmat(_C32, 128)), _dot(x, cmat(_S32, 128))

    def nyq_4():
        if 3 not in nyq:
            return
        xc, xs = nyq.pop(3)
        tr, ti = xc[:N2] - xs[N2:], xc[N2:] + xs[:N2]
        c, s = tw_v[0], tw_v[1]
        t = jnp.concatenate([tr * c - ti * s, ti * c + tr * s], axis=0).astype(BF16)
        yn_v[...] = _dot(_as_bf16(gt_v[0, 0:N2 // 2, :]), t)

    def a_inv_s(a, p):
        gm = _as_bf16(gt_v[2 * a + p])
        for t in range(2):
            row = yrow(t, 2 * a + p)
            r = _dot(gm, pltpu.bitcast(arena[row:row + 2 * N2, :], F32).astype(BF16))
            e_v[a % 2, 2 * t, N2 * p:N2 * p + N2, :] = r[:N2]
            e_v[a % 2, 2 * t + 1, N2 * p:N2 * p + N2, :] = r[N2:]

    def a_inv_d(a):
        even = (lane2 & 1) == 0
        ere, eim = e_v[a % 2, 0], pltpu.roll(e_v[a % 2, 1], 1, 1)
        yn = yn_v[...]
        nq = jnp.concatenate([pltpu.roll(yn, (1 - n1) % 128, 1) if n1 != 1 else yn
                              for n1 in (2 * a, 2 * a + 1)], axis=0)
        ea = _dot(jnp.where(lane2 == 1, nq, jnp.where(even, ere, eim)), cmat(_IA, 128))
        eb = _dot(jnp.where(even, eim, ere), cmat(_IB, 128))
        ore, oim = e_v[a % 2, 2], e_v[a % 2, 3] * lane_sign
        k1 = _dot(ore + oim, cmat(_I1, 128))
        v0, v1 = k1 + _dot(oim, cmat(_I2, 128)), k1 - _dot(ore, cmat(_I3, 128))
        pp, qq = ea + eb, ea - eb
        for c, y in enumerate((pp + v0, qq + v1, pp - v0, qq - v1)):
            for p in range(2):
                yp[c, pl.ds(2 * a + p, N2, stride=YP), :] = y[N2 * p:N2 * p + N2]

    fast = [pair for lo, hi in plan.get("fast", [[0, 25], [43, 48]]) for pair in range(lo, hi)]
    main = []
    for pair in range(48):
        if pair in fast and any(lo <= pair < hi for lo, hi in plan.get("big", [[15, 21]])):
            main += [P(project_big, pair, c, part) for c in range(2) for part in range(4)]
        elif pair in fast:
            main += [P(project, pair, c, half) for c in range(4) for half in range(2)]
        else:
            main += [P(project_plain, pair, n, c) for n in range(2) for c in range(4)]
    side = {}

    def spread(tasks, lo, hi, clear=1, odd=False):
        slots = [i for i in range(lo, hi) if not any(0 <= i - p < clear for p in waits)]
        if odd:
            slots = [i for i in slots if i % 2 == 1 or (i - 1) // 8 not in fast]
        for j, f in enumerate(tasks):
            side.setdefault(slots[(j * len(slots)) // len(tasks)], []).append(f)

    at = lambda name, *default: plan.get(name, default)
    wpos = plan.get("wpos", [20, 41, 77, 126, 167, 201, 238, 290])
    waits = dict(zip(wpos, ([1], [2], [3, 4], [5, "ax"], [6, "g", "cd"], ["wr", "wi", "tw", 7], [8, "gt", 9], [10, 11])))
    for pos, done in waits.items():
        spread([P(sync, done, [])], pos, pos + 1, 0)
    first = {1: wpos[0], 2: wpos[1], 3: wpos[2], 6: wpos[4], 7: wpos[5], 8: wpos[6], 10: wpos[7]}
    for u in range(1, 12):
        spread([P(stage_piece, u, k + 8 * half) for k in range(8) for half in range(2)],
               first.get(u, 32 * u - 31), 32 * u - 1, odd=plan.get("odd", False))
    for pair in range(1, 48):
        spread([P(relayout, pair, k, pair in fast) for k in range(8)], 8 * pair - 8, 8 * pair, plan.get("rclear", 1))
    spread([P(a_decimate, n2) for n2 in range(N2)], *at("dec", 126, 166), odd=plan.get("odd_dec", False))
    tasks = [P(a_fwd_d, 0)]
    for a in range(16):
        tasks += ([P(a_fwd_d, a + 1)] if a + 1 < 16 else []) + [P(a_fwd_s, a, 0), P(a_fwd_s, a, 1)]
    spread(tasks, *at("fwd", 167, 201))
    groups = [(t, j) for j in range(8) for t in range(2)]
    spread([P(filter_transpose, q, c) for c in range(16) for q in range(2)], *at("tr", 201, 230))
    spread([P(fft_p1, t, j, j1) for t, j in groups for j1 in range(8)], *at("p1", 202, 238))
    spread([P(fft_p2, t, j, r) for r in range(4) for t, j in groups], *at("p2", 238, 310, 2))
    spread([P(fft_p3, t, j, half) for t, j in groups for half in range(2)], *at("p3", 310, 343))
    spread([nyq_1, nyq_2, nyq_3], *at("nyq", 203, 218))
    spread([nyq_4], *at("nyq4", 242, 243))
    tasks = [P(a_inv_s, 0, 0), P(a_inv_s, 0, 1)]
    for a in range(16):
        tasks += ([P(a_inv_s, a + 1, 0), P(a_inv_s, a + 1, 1)] if a + 1 < 16 else []) + [P(a_inv_d, a)]
    spread(tasks, *at("inv", 344, 383))

    wos, w0 = [("wo", n) for n in range(4)], [("w0", q) for q in range(4)]
    if not prologue:
        main, side = [], {}
        sync([], ["bx1", "mem"])
        sync(["bx1", "mem"], [])
    sync([], ["bx0", *w0, 1, 2, 3, 4, 5, "ax", 6, "g", "cd", "wr", "wi", "tw", 7, 8, "gt", 9, 10, 11, *wos, "bx1", "mem"]
         if prologue else ["bx0", *w0])
    sync(["bx0"], [])
    token_sums()
    def run(tasks):
        pending = [g for g in (f() for f in tasks) if g is not None and next(g, 0) is None]
        for g in pending:
            next(g, None)

    for q in range(4):
        sync([w0[q]], [])
        run([P(stage_piece, 0, piece) for piece in range(4 * q, 4 * q + 4)])
    for k in range(0, 8, 2):
        run([P(relayout, 0, k + i, 0 in fast) for i in range(2)])
    for i, f in enumerate(main):
        if window and not window[0] <= i < window[1]:
            continue
        run(side.get(i, []))
        f()
    if prologue:
        sync([*wos, "bx1", "mem"], [])

    scale = DH ** -0.5 * LOG2E

    def step(s, m):
        rows = lax.broadcasted_iota(jnp.int32, (2 * L, 128), 0)
        cols = lax.broadcasted_iota(jnp.int32, (2 * L, 128), 1)
        rl = jnp.where(rows >= L, rows - L, rows)
        cl = jnp.where(cols >= L, cols - L, cols)
        same = ((rows >= L) == (cols >= L)) & (cols < 2 * L)
        valid = same & ((rl < M) | (rl >= cl))
        fill = jnp.where(same, -1e9 * LOG2E, -jnp.inf).astype(F32)
        aligned = (lambda v, n: v) if isinstance(s, int) else pl.multiple_of
        xs = bx_v[pl.ds(aligned(R0 + s * RX, 8), RX), :].astype(F32)
        wpos = aligned((s * RX) % RING, 8)
        rpos = aligned((RING - R0 + s * SEG) % RING, SEG)
        hk = [jnp.concatenate([xs[:, 128 * k:128 * (k + 1)], m[k]], axis=0) for k in range(4)]
        h4 = jnp.concatenate(hk, axis=1)

        def put(w, hd, y):
            g, i = divmod(hd, 8)
            mems[g][8 * w + i] = y[RX:]
            rings[g][8 * w + i, pl.ds(wpos, RX), :] = y[:RX]

        def get(w, hd):
            g, i = divmod(hd, 8)
            return [mems[g][8 * w + i], rings[g][8 * w + i, pl.ds(rpos, SEG), :]]

        def proj(w, hd):
            put(w, hd, _dot(h4, weight(w, hd)))

        part = {}

        def proj_k(tiles, k):
            for w, hd in tiles:
                y = _dot(hk[k], weight(w, hd, 64 * k, 64 * k + 64))
                part[w, hd] = y if k == 0 else part[w, hd] + y
                if k == 3:
                    put(w, hd, part.pop((w, hd)))

        def keys(w, j):
            pad = jnp.zeros((128 - 2 * L, DH), F32)
            return jnp.concatenate(get(w, 2 * j) + get(w, 2 * j + 1) + [pad], axis=0).astype(BF16)

        def scores(j):
            q2 = jnp.concatenate(get(0, 2 * j) + get(0, 2 * j + 1), axis=0)
            s_scr[j // 4][j % 4] = lax.dot_general(q2, keys(1, j), (((1,), (1,)), ((), ())),
                                                   preferred_element_type=F32)

        def softmax(j):
            sc = jnp.where(valid, s_scr[j // 4][j % 4] * scale, fill)
            e = jnp.exp2(sc - jnp.max(sc, axis=-1, keepdims=True))
            total = jnp.sum(e, axis=-1, keepdims=True)
            inv = pltpu.reciprocal(total, approx=True)
            inv = inv * (2.0 - total * inv)
            p_scr[j // 4][j % 4] = (e * inv).astype(BF16)

        def pv(j):
            o2 = _dot(p_scr[j // 4][j % 4], keys(2, j))
            o_scr[j // 4][2 * (j % 4)] = o2[:L]
            o_scr[j // 4][2 * (j % 4) + 1] = o2[L:]

        accs = [None] * 4

        def wo(g, n):
            lhs = jnp.concatenate([o_scr[g // 2][4 * (g % 2) + i] for i in range(4)], axis=1)
            y = _dot(lhs, wo_st[n, 512 * g:512 * g + 512, :])
            accs[n] = y if accs[n] is None else accs[n] + y

        qk = plan.get("qk", "qblock")
        if qk == "kblock":
            order = [(w, hd) for g in range(4) for w in (1, 0) for hd in range(8 * g, 8 * g + 8)]
        elif qk == "qblock":
            order = [(w, hd) for g in range(4) for w in (0, 1) for hd in range(8 * g, 8 * g + 8)]
        else:
            order = [(w, hd) for hd in range(H) for w in ((0, 1) if qk == "qk" else (1, 0))]
        order += [(2, hd) for hd in range(H)]

        main = [P(proj_k, order[:4], k) for k in range(4)] + [P(proj, *t) for t in order[4:]]
        wmode = plan.get("wmode", 0)
        if wmode == 0:
            main += [P(wo, g, n) for g in range(8) for n in range(3)] + [P(wo, g, 3) for g in range(8)]
        elif wmode == 1:
            main += [P(wo, g, n) for g in range(4) for n in range(4)]
            main += [P(wo, g, n) for g in range(4, 8) for n in range(3)] + [P(wo, g, 3) for g in range(4, 8)]
        elif wmode == 2:
            main += [P(wo, g, n) for g in range(6) for n in range(4)] + [P(wo, g, n) for n in range(4) for g in (6, 7)]
        else:
            main += [P(wo, g, n) for g in range(4) for n in range(4)] + [P(wo, g, n) for n in range(4) for g in range(4, 8)]
        extra = {}
        for g in range(4):
            pos = 16 * (g + 1) + (s_lag[g] if isinstance(s_lag, list) else s_lag)
            for jj in range(4):
                extra.setdefault(pos, []).append(P(scores, 4 * g + jj))
            for jj in range(4):
                extra.setdefault(pos + sm_start + sm_gap * jj, []).append(P(softmax, 4 * g + jj))
            pos = 64 + 8 * (g + 1) + (a_lag[g] if isinstance(a_lag, list) else a_lag if g < 3 else a_last)
            for jj in range(4):
                extra.setdefault(pos, []).append(P(pv, 4 * g + jj))
        for i, f in enumerate(main):
            for e in extra.get(i, []):
                e()
            f()
        rows = pl.ds(aligned(s * SEG, SEG), SEG)
        for c in range(4):
            out_v[rows, 128 * c:128 * c + 128] = yp[c, pl.ds(aligned(s * YP, 8), SEG), :].astype(BF16)
            out_v[rows, D + 128 * c:D + 128 * c + 128] = accs[c][M:].astype(BF16)
        return [a[:M] for a in accs]

    def out_copy(s):
        rows = pl.ds(s * SEG if isinstance(s, int) else pl.multiple_of(s * SEG, SEG), SEG)
        return pltpu.make_async_copy(out_v.at[rows], out_hbm.at[rows], out_sems)

    peel = nseg % unroll

    def body(i, m):
        for u in range(unroll):
            m = step(peel + i * unroll + u, m)
            out_copy(peel + i * unroll + u).start()
        return m

    m0 = mem_v[...].astype(F32)
    if nseg == 0:
        def keep(i, c):
            rows = pl.ds(pl.multiple_of(i * 16, 16), 16)
            out_v[rows, 0:128] = (sum(r[i, rows, :] for r in rings) + yp[0, rows, :] + y0_v[0, i, rows, :]
                                  + pltpu.bitcast(f_v[0, rows, :] | arena[rows, :], F32)).astype(BF16)
            return c
        lax.fori_loop(0, 4, keep, 0)
        out_copy(0).start()
        out_copy(0).wait()
        return
    m = [m0[:, 128 * k:128 * (k + 1)] for k in range(4)]
    for s in range(peel):
        m = step(s, m)
        out_copy(s).start()
    lax.fori_loop(0, nseg // unroll, body, m)

    def drain(i, c):
        out_copy(i).wait()
        return c

    lax.fori_loop(0, nseg, drain, 0)


def make(unroll=4, s_lag=9, a_lag=6, a_last=5, sm_start=3, sm_gap=2, flags=None, interpret=False, nseg=NSEG, prologue=True, window=None, plan=None):
    vm = pltpu.VMEM
    scratch = [
        vm((S, D), BF16), vm((D // 2 + 1, S), BF16), vm((D // 2 + 1, S), BF16), vm((S, D), BF16), vm((M, D), BF16),
        vm((12, D, 8, DH), BF16), vm((4, H * DH, 128), BF16),
        vm(_CD.shape, U32), vm(_G.shape, U32), vm(_GT.shape, U32), vm(_TW.shape, F32),
        vm((A_ROWS, 128), U32), vm((2, S, 128), U32), vm((2 * 5 * 128, 128), U32), vm((2 * TMP_ROWS + 16, 128), U32), vm((7, 2, R0 // 4, 128), U32), vm((4, R0 // 2, 128), U32), vm((2, 4, 2 * N2, 128), F32),
        vm((2, N1, 2 * N2, 128), F32), vm((N2, 128), F32), vm((N2, 128), F32), vm((4, YP * N2 + 40, 128), F32),
        vm((S, 2 * D), BF16),
    ]
    scratch += [vm((24, RING, DH), F32)] * 4 + [vm((24, M, DH), F32)] * 4
    scratch += [vm((4, 2 * L, 128), F32)] * 4 + [vm((4, 2 * L, 128), BF16)] * 4 + [vm((8, L, DH), F32)] * 4
    scratch += [pltpu.SemaphoreType.DMA((29,)), pltpu.SemaphoreType.DMA(())]
    kern = functools.partial(_kernel, unroll=unroll, s_lag=s_lag, a_lag=a_lag, a_last=a_last,
                             sm_start=sm_start, sm_gap=sm_gap, nseg=nseg, prologue=prologue,
                             window=window, plan=plan or {})

    @jax.jit
    def f(A_x, A_w_r, A_w_i, B_x, B_mem0, B_Wq, B_Wk, B_Wv, B_Wo):
        out = pl.pallas_call(
            kern,
            out_shape=jax.ShapeDtypeStruct((S, 2 * D), BF16),
            in_specs=[pl.BlockSpec(memory_space=pltpu.SMEM)] + [pl.BlockSpec(memory_space=pltpu.HBM)] * 13,
            out_specs=pl.BlockSpec(memory_space=pltpu.HBM),
            scratch_shapes=scratch,
            compiler_params=pltpu.CompilerParams(vmem_limit_bytes=120 * 1024 * 1024, flags=flags),
            interpret=interpret,
        )(np.zeros((1,), np.int32), A_x.reshape(S, D), A_w_r.T, A_w_i.T, B_x.reshape(S, D), B_mem0.reshape(M, D), B_Wq, B_Wk, B_Wv,
          B_Wo.reshape(H * DH, D), _CD, _G, _GT, _TW)
        return out.reshape(1, S, 2 * D)

    return f


_run = make()


def pallas_concat_heads__spectral_gfnet__memory_aug_recurrent_mem_tr__prompt_kernel(
        A_x, A_w_r, A_w_i, B_x, B_mem0, B_Wq, B_Wk, B_Wv, B_Wo, B_seg_len):
    assert int(B_seg_len) == SEG and A_x.shape == (1, S, D) and B_Wq.shape == (D, H, DH)
    return _run(A_x, A_w_r, A_w_i, B_x, B_mem0, B_Wq, B_Wk, B_Wv, B_Wo)
```

```python
import functools

import jax
import jax.numpy as jnp
import numpy as np
from jax import lax
from jax.experimental import pallas as pl
from jax.experimental.pallas import tpu as pltpu

F32, BF16, U32 = jnp.float32, jnp.bfloat16, jnp.uint32
P = functools.partial

S, D = 2048, 512
H, DH, M, SEG = 32, 128, 8, 32
L = M + SEG
NSEG = S // SEG
N1, N2 = 32, 64
R0, RX = 512, 24
RING = 576
UNROLL = 7
XP, YP, TP = 17, 40, 9
LOG2E = 1.4426950408889634

TILE = D // 2
TMP_ROWS = TP * TILE
XP_ROWS = XP * N2 + 24
A_WEIGHTS = 0
A_TMP = A_WEIGHTS + 3 * H * TILE
A_SUMS = A_TMP + 2 * TMP_ROWS + 16
A_XP = A_SUMS + 2 * 5 * 128
A_Y = A_XP + 4 * XP_ROWS
A_ROWS = A_Y + 2 * N1 * 2 * N2


def _pack_bf16(a):
    u = np.ascontiguousarray(a, dtype=np.float32).view(np.uint32)
    b = ((u + 0x7FFF + ((u >> 16) & 1)) >> 16).astype(np.uint32)
    return b[..., 0::2, :] | (b[..., 1::2, :] << 16)


def _dft_constants():
    lane = np.arange(128)
    angle = lambda k: 2 * np.pi * np.outer(lane, k) / D
    even = lane % 2 == 0
    re, im = np.cos(angle(2 * lane)), -np.sin(angle(2 * ((lane - 1) % 128)))
    fa, fb = np.where(even[None, :], re, im), np.where(even[None, :], im, re)
    fa[:, 1] = np.cos(np.pi * lane)
    p, q = np.cos(angle(2 * lane + 1)), -np.sin(angle(2 * lane + 1))
    sign = np.where(even, -1.0, 1.0)[None, :]
    f2, f3 = q - sign * p, p + sign * q
    scale = 2.0 / (S * D)
    once = np.where(lane < 2, 0.5, 1.0)[None, :]
    inverse = [(m * scale).T for m in (fa * once, fb, p, sign * f2, f3)]
    a32 = 2 * np.pi * np.outer(np.arange(N1), np.arange(N1)) / N1
    c32, s32 = np.zeros((128, 128)), np.zeros((128, 128))
    c32[:N1, :N1], s32[:N1, :N1] = np.cos(a32), np.sin(a32)
    model_axis = np.concatenate([fa, fb, p, f2, f3] + inverse + [c32, s32], axis=0)
    k2 = np.arange(N2)
    g = np.zeros((N1, 2 * N2, 2 * N2))
    for n1 in range(N1):
        a = 2 * np.pi * np.outer(k2, n1 + N1 * k2) / S
        g[n1] = np.block([[np.cos(a), np.sin(a)], [-np.sin(a), np.cos(a)]])
    a = 2 * np.pi * np.outer(k2, np.arange(N1)) / S
    twiddle = np.zeros((2, N2, 128), np.float32)
    twiddle[0, :, :N1], twiddle[1, :, :N1] = np.cos(a), np.sin(a)
    return _pack_bf16(model_axis), _pack_bf16(g), _pack_bf16(g.transpose(0, 2, 1)), twiddle


_CD, _G, _GT, _TW = _dft_constants()
_FA, _FB, _F1, _F2, _F3, _IA, _IB, _I1, _I2, _I3, _C32, _S32 = range(12)


def _dot(a, b):
    return jnp.dot(a, b, preferred_element_type=F32)


def _as_bf16(words):
    return pltpu.bitcast(words, BF16)


def _low(words):
    return pltpu.bitcast(words << 16, F32)


def _high(words):
    return pltpu.bitcast(words & jnp.uint32(0xFFFF0000), F32)


def _add(a, b):
    return a[0] + b[0], a[1] + b[1]


def _sub(a, b):
    return a[0] - b[0], a[1] - b[1]


def _add_i(a, b):
    return a[0] - b[1], a[1] + b[0]


def _sub_i(a, b):
    return a[0] + b[1], a[1] - b[0]


def _twiddle(a, e, n):
    e %= n
    if e == 0:
        return a
    if 4 * e == n:
        return a[1], -a[0]
    if 4 * e == 3 * n:
        return -a[1], a[0]
    if 2 * e == n:
        return -a[0], -a[1]
    c, s = float(np.cos(2 * np.pi * e / n)), float(np.sin(2 * np.pi * e / n))
    if (8 * e) % n == 0:
        h = abs(c)
        if c > 0 and s > 0:
            return (a[0] + a[1]) * h, (a[1] - a[0]) * h
        if c < 0 and s > 0:
            return (a[1] - a[0]) * h, (a[0] + a[1]) * (-h)
        if c < 0 and s < 0:
            return (a[0] + a[1]) * (-h), (a[0] - a[1]) * h
        return (a[0] - a[1]) * h, (a[0] + a[1]) * h
    return a[0] * c + a[1] * s, a[1] * c - a[0] * s


def _dft4(z, forward):
    a, b, c, d = _add(z[0], z[2]), _sub(z[0], z[2]), _add(z[1], z[3]), _sub(z[1], z[3])
    if forward:
        return [_add(a, c), _sub_i(b, d), _sub(a, c), _add_i(b, d)]
    return [_add(a, c), _add_i(b, d), _sub(a, c), _sub_i(b, d)]


def _fft8(z):
    ev = _dft4([_add(z[j], z[j + 4]) for j in range(4)], True)
    d = [_sub(z[j], z[j + 4]) for j in range(4)]
    d1, d3 = _twiddle(d[1], 1, 8), _twiddle(d[3], 3, 8)
    a, b, c, e = _sub_i(d[0], d[2]), _add_i(d[0], d[2]), _add(d1, d3), _sub(d1, d3)
    od = [_add(a, c), _sub_i(b, e), _sub(a, c), _add_i(b, e)]
    return [ev[m // 2] if m % 2 == 0 else od[m // 2] for m in range(8)]


def _ifft8(x):
    ev = _dft4([x[0], x[2], x[4], x[6]], False)
    od = _dft4([x[1], x[3], x[5], x[7]], False)
    o1, o3 = _twiddle(od[1], -1, 8), _twiddle(od[3], -3, 8)
    lo = [_add(ev[0], od[0]), _add(ev[1], o1), _add_i(ev[2], od[2]), _add(ev[3], o3)]
    hi = [_sub(ev[0], od[0]), _sub(ev[1], o1), _sub_i(ev[2], od[2]), _sub(ev[3], o3)]
    return lo + hi


def _run(tasks):
    pending = [g for g in (f() for f in tasks) if g is not None and next(g, 0) is None]
    for g in pending:
        next(g, None)


def _kernel(zero_ref, ax_hbm, wr_hbm, wi_hbm, bx_hbm, mem_hbm, wq_hbm, wk_hbm, wv_hbm, wo_hbm,
            cd_hbm, g_hbm, gt_hbm, tw_hbm, out_hbm,
            ax_v, wr_v, wi_v, bx_v, mem_v, w_v, wo_v, cd_v, g_v, gt_v, tw_v,
            arena, filt_v, xsum_v, x_v, e_v, y_v, nyq_in, nyq_out, ya_v, out_v, *rest):
    rings, mems, s_v, p_v, o_v = [rest[4 * i:4 * i + 4] for i in range(5)]
    sems, out_sem = rest[20:]
    pin = pl.multiple_of(zero_ref[0], 8)

    copies = {}

    def add_copy(name, src, dst):
        copies[name] = pltpu.make_async_copy(src, dst, sems.at[len(copies)])

    def wait(*names):
        for name in names:
            copies[name].wait()

    for u in range(1, 12):
        add_copy(u, (wq_hbm, wk_hbm, wv_hbm)[u // 4].at[:, pl.ds(8 * (u % 4), 8), :], w_v.at[u])
    w0 = [("w0", q) for q in range(4)]
    for q in range(4):
        add_copy(w0[q], wq_hbm.at[pl.ds(128 * q, 128), pl.ds(0, 8), :], w_v.at[0, pl.ds(128 * q, 128)])
    add_copy("bx0", bx_hbm.at[pl.ds(0, R0)], bx_v.at[pl.ds(0, R0)])
    add_copy("bx1", bx_hbm.at[pl.ds(R0, S - R0)], bx_v.at[pl.ds(R0, S - R0)])
    wo = [("wo", n) for n in range(4)]
    for n in range(4):
        add_copy(wo[n], wo_hbm.at[:, pl.ds(128 * n, 128)], wo_v.at[n])
    for name, src, dst in (("ax", ax_hbm, ax_v), ("wr", wr_hbm, wr_v), ("wi", wi_hbm, wi_v), ("mem", mem_hbm, mem_v),
                           ("cd", cd_hbm, cd_v), ("g", g_hbm, g_v), ("gt", gt_hbm, gt_v), ("tw", tw_hbm, tw_v)):
        add_copy(name, src, dst)

    lane = lax.broadcasted_iota(jnp.int32, (N2, 128), 1)
    lane2 = lax.broadcasted_iota(jnp.int32, (2 * N2, 128), 1)
    lane_sign = jnp.where((lane2 & 1) == 0, -1.0, 1.0).astype(F32)

    def const(i):
        return _as_bf16(cd_v[64 * i:64 * i + 64, :])

    def tile_row(t):
        return A_WEIGHTS + TILE * t

    def weight(t, lo=0, hi=TILE):
        return _as_bf16(arena[tile_row(t) + lo:tile_row(t) + hi, :])

    def stage(u, piece):
        words = pltpu.bitcast(w_v[u, 32 * piece:32 * piece + 32].reshape(32 * 8, DH), U32)
        yield
        for j in range(16):
            row = A_TMP + (u % 2) * TMP_ROWS + TP * (16 * piece + j)
            arena[pl.ds(pin + row, 8), :] = words[8 * j:8 * j + 8]

    def relayout(pair, k, sums):
        u, i = divmod(pair, 4)
        halves = [[arena[pl.ds(A_TMP + (u % 2) * TMP_ROWS + TP * (128 * half + 16 * k) + i + 4 * q, 16, stride=TP), :]
                   for q in range(2)] for half in range(2)]
        yield
        for half, (ev, od) in enumerate(halves):
            row = (0 if sums else pin) + tile_row(2 * pair) + 128 * half + 16 * k
            arena[pl.ds(row, 16), :] = (ev & jnp.uint32(0xFFFF)) | (od << 16)
            arena[pl.ds(row + TILE, 16), :] = (ev >> 16) | (od & jnp.uint32(0xFFFF0000))
        if sums:
            b11, b12, b21, b22 = [(f(ev), f(od)) for ev, od in halves for f in (_low, _high)]
            for n, t in enumerate((_add(b11, b22), _sub(b12, b22), _sub(b21, b11), _add(b11, b12), _add(b21, b22))):
                ev, od = [pltpu.bitcast(v, U32) + jnp.uint32(0x8000) for v in t]
                arena[pl.ds(pin + A_SUMS + ((pair % 2) * 5 + n) * 128 + 16 * k, 16), :] = (
                    (ev >> 16) | (od & jnp.uint32(0xFFFF0000)))

    def token_sums():
        def quad(r, k):
            return bx_v[256 * r:256 * r + 256, 256 * k:256 * k + 256].astype(F32)

        for k in range(4):
            x_v[k] = pltpu.bitcast(bx_v[0:R0, 128 * k:128 * k + 128], U32)
        a11, a12, a21, a22 = quad(0, 0), quad(0, 1), quad(1, 0), quad(1, 1)
        for i, t in enumerate((a11 + a22, a21 + a22, a11, a22, a11 + a12, a21 - a11, a12 - a22)):
            for k in range(2):
                xsum_v[i, k] = pltpu.bitcast(t[:, 128 * k:128 * k + 128].astype(BF16), U32)

    def put_tokens(t, row, y):
        w, head = divmod(t, H)
        rings[head // 8][8 * w + head % 8, pl.ds(RING - R0 + row, y.shape[0]), :] = y

    def project(t, c):
        lhs = jnp.concatenate([_as_bf16(x_v[k, 64 * c:64 * c + 64, :]) for k in range(4)], axis=1)
        put_tokens(t, 128 * c, _dot(lhs, weight(t)))

    def product(pair, i, c, rows):
        words = slice(rows // 2 * c, rows // 2 * (c + 1))
        lhs = jnp.concatenate([_as_bf16(xsum_v[i - 1, k, words, :]) for k in range(2)], axis=1)
        if i == 2:
            return _dot(lhs, weight(2 * pair, 0, 128))
        if i == 5:
            return _dot(lhs, weight(2 * pair + 1, 128, 256))
        row = A_SUMS + ((pair % 2) * 5 + (1, 3, 4, 6, 7).index(i)) * 128
        return _dot(lhs, _as_bf16(arena[row:row + 128, :]))

    carry = []

    def strassen64(pair, c, part):
        m = lambda i: product(pair, i, c, 64)
        if part == 0:
            m3, m5, m2, m4 = m(3), m(5), m(2), m(4)
            put_tokens(2 * pair + 1, 64 * c, m3 + m5)
            put_tokens(2 * pair, 256 + 64 * c, m2 + m4)
            carry.append((m4 - m5, m3 - m2))
        else:
            t11, t22 = carry.pop()
            m1, m7, m6 = m(1), m(7), m(6)
            put_tokens(2 * pair, 64 * c, m1 + m7 + t11)
            put_tokens(2 * pair + 1, 256 + 64 * c, m1 + m6 + t22)

    def strassen128(pair, c, part):
        m = lambda i: product(pair, i, c, 128)
        if part == 0:
            m3, m5 = m(3), m(5)
            put_tokens(2 * pair + 1, 128 * c, m3 + m5)
            carry.append((m5, m3))
        elif part == 1:
            m5, m3 = carry.pop()
            m2, m4 = m(2), m(4)
            put_tokens(2 * pair, 256 + 128 * c, m2 + m4)
            carry.append((m4 - m5, m3 - m2))
        elif part == 2:
            t11, t22 = carry.pop()
            m1, m7 = m(1), m(7)
            put_tokens(2 * pair, 128 * c, m1 + m7 + t11)
            carry.append(m1 + t22)
        else:
            m6 = m(6)
            put_tokens(2 * pair + 1, 256 + 128 * c, m6 + carry.pop())

    def decimate(n2):
        yield
        for c in range(4):
            arena[pl.ds(pin + A_XP + c * XP_ROWS + XP * n2, 16), :] = pltpu.bitcast(
                ax_v[32 * n2:32 * n2 + 32, 128 * c:128 * c + 128], U32)

    def forward_model_axis(a):
        xs = []
        for c in range(4):
            words = arena[pl.ds(A_XP + c * XP_ROWS + a, N2, stride=XP), :]
            xs.append(jnp.concatenate([_low(words), _high(words)], axis=0))
        u0, u1, v0, v1 = xs[0] + xs[2], xs[1] + xs[3], xs[0] - xs[2], xs[1] - xs[3]
        e_v[a % 2, 0] = _dot(u0 + u1, const(_FA))
        e_v[a % 2, 1] = _dot(u0 - u1, const(_FB))
        k1 = _dot(v0 + v1, const(_F1))
        e_v[a % 2, 2] = k1 - _dot(v1, const(_F3))
        e_v[a % 2, 3] = k1 * lane_sign + _dot(v0, const(_F2))

    def forward_sequence_axis(a, p):
        n1 = 2 * a + p
        ea, eb, ore, oim = [e_v[a % 2, q, N2 * p:N2 * p + N2, :] for q in range(4)]
        even = (lane & 1) == 0
        ere = jnp.where(even, ea, eb)
        eim = pltpu.roll(jnp.where(even, eb, jnp.where(lane == 1, 0.0, ea)), 127, 1)
        nyquist = pltpu.roll(ea, (n1 - 1) % 128, 1) if n1 != 1 else ea
        nyq_in[...] = jnp.where(lane == n1, nyquist, 0.0 if n1 == 0 else nyq_in[...])
        g = _as_bf16(g_v[n1])
        y_v[0, n1] = _dot(g, jnp.concatenate([ere, eim], axis=0).astype(BF16))
        y_v[1, n1] = _dot(g, jnp.concatenate([ore, oim], axis=0).astype(BF16))

    def transpose_filter(q, c):
        filt_v[q, 128 * c:128 * c + 128, :] = pltpu.bitcast((wr_v, wi_v)[q][0:256, 128 * c:128 * c + 128], U32).T

    def spectrum_row(t, n):
        return A_Y + (t * N1 + n) * 2 * N2

    def load(t, n, j):
        row = spectrum_row(t, n) + 8 * j
        return pltpu.bitcast(arena[row:row + 8, :], F32), pltpu.bitcast(arena[row + N2:row + N2 + 8, :], F32)

    def store(t, n, j, z):
        row = spectrum_row(t, n) + 8 * j
        arena[pl.ds(pin + row, 8), :] = pltpu.bitcast(z[0], U32)
        arena[pl.ds(pin + row + N2, 8), :] = pltpu.bitcast(z[1], U32)

    def fft_first(t, j, j1):
        z = [(y_v[t, j1 + 8 * q, 8 * j:8 * j + 8, :], y_v[t, j1 + 8 * q, N2 + 8 * j:N2 + 8 * j + 8, :])
             for q in range(4)]
        o = _dft4(z, True)
        yield
        for r in range(4):
            store(t, 8 * r + j1, j, _twiddle(o[r], r * j1, N1))

    def fft_filter(t, j, r):
        x = _fft8([load(t, 8 * r + j1, j) for j1 in range(8)])
        for m in range(8):
            row = N2 * (4 * m + r) + 8 * j
            fr, fi = [(_low, _high)[t](filt_v[q, row:row + 8, :]) for q in range(2)]
            x[m] = (x[m][0] * fr - x[m][1] * fi, x[m][0] * fi + x[m][1] * fr)
        z = _ifft8(x)
        yield
        for j1 in range(8):
            store(t, 8 * r + j1, j, z[j1])

    def fft_last(t, j, half):
        cols = range(4 * half, 4 * half + 4)
        o = {j1: [load(t, 8 * r + j1, j) for r in range(4)] for j1 in cols}
        yield
        for j1 in cols:
            z = _dft4([_twiddle(o[j1][r], -r * j1, N1) for r in range(4)], False)
            for q in range(4):
                store(t, j1 + 8 * q, j, z[q])

    nyq = []

    def nyquist_1():
        rhs = jnp.concatenate([nyq_in[...], jnp.zeros((N2, 128), F32)], axis=0).astype(BF16)
        nyq.append(_dot(_as_bf16(g_v[0]), rhs))

    def nyquist_2():
        y = nyq.pop()
        c, s = tw_v[0], tw_v[1]
        y = jnp.concatenate([y[:N2] * c + y[N2:] * s, y[N2:] * c - y[:N2] * s], axis=0)
        nyq.append((_dot(y, const(_C32)), _dot(y, const(_S32))))

    def nyquist_filter(ref):
        row = lax.broadcasted_iota(jnp.int32, (N1, 128), 0)
        f = jnp.zeros((N1, 128), F32)
        for c in range(16):
            v = jnp.broadcast_to(ref[256:257, 128 * c:128 * c + 128].astype(F32), (8, 128))
            f = jnp.where(row == 2 * c, jnp.concatenate([v] * 4, axis=0), f)
            f = jnp.where(row == 2 * c + 1, jnp.concatenate([pltpu.roll(v, 64, 1)] * 4, axis=0), f)
        return jnp.concatenate([f, jnp.zeros((128 - N1, 128), F32)], axis=0).T[:N2]

    def nyquist_3():
        yc, ys = nyq.pop()
        xr, xi = yc[:N2] + ys[N2:], yc[N2:] - ys[:N2]
        fr, fi = nyquist_filter(wr_v), nyquist_filter(wi_v)
        x = jnp.concatenate([xr * fr - xi * fi, xr * fi + xi * fr], axis=0)
        nyq.append((_dot(x, const(_C32)), _dot(x, const(_S32))))

    def nyquist_4():
        xc, xs = nyq.pop()
        tr, ti = xc[:N2] - xs[N2:], xc[N2:] + xs[:N2]
        c, s = tw_v[0], tw_v[1]
        t = jnp.concatenate([tr * c - ti * s, ti * c + tr * s], axis=0).astype(BF16)
        nyq_out[...] = _dot(_as_bf16(gt_v[0, 0:N2 // 2, :]), t)

    def inverse_sequence_axis(a, p):
        g = _as_bf16(gt_v[2 * a + p])
        for t in range(2):
            row = spectrum_row(t, 2 * a + p)
            r = _dot(g, pltpu.bitcast(arena[row:row + 2 * N2, :], F32).astype(BF16))
            e_v[a % 2, 2 * t, N2 * p:N2 * p + N2, :] = r[:N2]
            e_v[a % 2, 2 * t + 1, N2 * p:N2 * p + N2, :] = r[N2:]

    def inverse_model_axis(a):
        even = (lane2 & 1) == 0
        ere, eim = e_v[a % 2, 0], pltpu.roll(e_v[a % 2, 1], 1, 1)
        yn = nyq_out[...]
        nyquist = jnp.concatenate([pltpu.roll(yn, (1 - n1) % 128, 1) if n1 != 1 else yn
                                   for n1 in (2 * a, 2 * a + 1)], axis=0)
        ea = _dot(jnp.where(lane2 == 1, nyquist, jnp.where(even, ere, eim)), const(_IA))
        eb = _dot(jnp.where(even, eim, ere), const(_IB))
        ore, oim = e_v[a % 2, 2], e_v[a % 2, 3] * lane_sign
        k1 = _dot(ore + oim, const(_I1))
        v0, v1 = k1 + _dot(oim, const(_I2)), k1 - _dot(ore, const(_I3))
        u0, u1 = ea + eb, ea - eb
        for c, y in enumerate((u0 + v0, u1 + v1, u0 - v0, u1 - v1)):
            for p in range(2):
                ya_v[c, pl.ds(2 * a + p, N2, stride=YP), :] = y[N2 * p:N2 * p + N2]

    main, fast = [], [*range(0, 25), *range(43, 48)]
    for pair in range(48):
        if pair not in fast:
            main += [P(project, 2 * pair + n, c) for n in range(2) for c in range(4)]
        elif 15 <= pair < 21:
            main += [P(strassen128, pair, c, part) for c in range(2) for part in range(4)]
        else:
            main += [P(strassen64, pair, c, part) for c in range(4) for part in range(2)]
    waits = {20: [1], 41: [2], 77: [3, 4], 126: [5, "ax"], 167: [6, "g", "cd"], 201: ["wr", "wi", "tw", 7],
             238: [8, "gt", 9], 290: [10, 11]}
    side = {slot: [P(wait, *names)] for slot, names in waits.items()}

    def spread(tasks, lo, hi, clear=1):
        free = [i for i in range(lo, hi) if not any(0 <= i - w < clear for w in waits)]
        slots = [free[(j * len(free)) // len(tasks)] for j in range(len(tasks))]
        for slot, task in zip(slots, tasks):
            side.setdefault(slot, []).append(task)
        return slots

    arrival = {name: slot for slot, names in waits.items() for name in names}
    staged = {u: spread([P(stage, u, k + 8 * half) for k in range(8) for half in range(2)],
                        max(arrival[u], 32 * u - 31), 32 * u - 1) for u in range(1, 12)}
    for pair in range(1, 48):
        slots = spread([P(relayout, pair, k, pair in fast) for k in range(8)], 8 * pair - 8, 8 * pair)
        assert pair < 4 or all(staged[pair // 4][2 * k + 1] < slots[k] for k in range(8))
    spread([P(decimate, n2) for n2 in range(N2)], 126, 166)
    tasks = [P(forward_model_axis, 0)]
    for a in range(16):
        tasks += [P(forward_model_axis, a + 1)] if a + 1 < 16 else []
        tasks += [P(forward_sequence_axis, a, 0), P(forward_sequence_axis, a, 1)]
    spread(tasks, 167, 201)
    groups = [(t, j) for j in range(8) for t in range(2)]
    spread([P(transpose_filter, q, c) for c in range(16) for q in range(2)], 201, 230)
    spread([P(fft_first, t, j, j1) for t, j in groups for j1 in range(8)], 202, 238)
    spread([P(fft_filter, t, j, r) for r in range(4) for t, j in groups], 238, 310, clear=2)
    spread([P(fft_last, t, j, half) for t, j in groups for half in range(2)], 310, 343)
    spread([nyquist_1, nyquist_2, nyquist_3], 203, 218)
    spread([nyquist_4], 242, 243)
    tasks = [P(inverse_sequence_axis, 0, 0), P(inverse_sequence_axis, 0, 1)]
    for a in range(16):
        tasks += [P(inverse_sequence_axis, a + 1, 0), P(inverse_sequence_axis, a + 1, 1)] if a + 1 < 16 else []
        tasks += [P(inverse_model_axis, a)]
    spread(tasks, 344, 383)

    for name in ["bx0", *w0, 1, 2, 3, 4, 5, "ax", 6, "g", "cd", "wr", "wi", "tw", 7, 8, "gt", 9, 10, 11, *wo,
                 "bx1", "mem"]:
        copies[name].start()
    wait("bx0")
    token_sums()
    for q in range(4):
        wait(w0[q])
        _run([P(stage, 0, piece) for piece in range(4 * q, 4 * q + 4)])
    for k in range(0, 8, 2):
        _run([P(relayout, 0, k + i, True) for i in range(2)])
    for slot, task in enumerate(main):
        _run(side.get(slot, []))
        task()
    wait(*wo, "bx1", "mem")

    def step(s, mem):
        rows = lax.broadcasted_iota(jnp.int32, (2 * L, 128), 0)
        cols = lax.broadcasted_iota(jnp.int32, (2 * L, 128), 1)
        row = jnp.where(rows >= L, rows - L, rows)
        col = jnp.where(cols >= L, cols - L, cols)
        same_head = ((rows >= L) == (cols >= L)) & (cols < 2 * L)
        visible = same_head & ((row < M) | (row >= col))
        masked = jnp.where(same_head, -1e9 * LOG2E, -jnp.inf).astype(F32)
        xs = bx_v[pl.ds(pl.multiple_of(R0 + s * RX, 8), RX), :].astype(F32)
        write_at = pl.multiple_of((s * RX) % RING, 8)
        read_at = pl.multiple_of((RING - R0 + s * SEG) % RING, SEG)
        hk = [jnp.concatenate([xs[:, 128 * k:128 * (k + 1)], mem[k]], axis=0) for k in range(4)]
        h = jnp.concatenate(hk, axis=1)

        def put(w, head, y):
            mems[head // 8][8 * w + head % 8] = y[RX:]
            rings[head // 8][8 * w + head % 8, pl.ds(write_at, RX), :] = y[:RX]

        def get(w, head):
            return [mems[head // 8][8 * w + head % 8], rings[head // 8][8 * w + head % 8, pl.ds(read_at, SEG), :]]

        def qkv(w, head):
            put(w, head, _dot(h, weight(w * H + head)))

        partial = {}

        def qkv_slice(tiles, k):
            for w, head in tiles:
                y = _dot(hk[k], weight(w * H + head, 64 * k, 64 * k + 64))
                partial[w, head] = y if k == 0 else partial[w, head] + y
                if k == 3:
                    put(w, head, partial.pop((w, head)))

        def stationary(w, j):
            pad = jnp.zeros((128 - 2 * L, DH), F32)
            return jnp.concatenate(get(w, 2 * j) + get(w, 2 * j + 1) + [pad], axis=0).astype(BF16)

        def scores(j):
            q = jnp.concatenate(get(0, 2 * j) + get(0, 2 * j + 1), axis=0)
            s_v[j // 4][j % 4] = lax.dot_general(q, stationary(1, j), (((1,), (1,)), ((), ())),
                                                 preferred_element_type=F32)

        def softmax(j):
            x = jnp.where(visible, s_v[j // 4][j % 4] * (DH ** -0.5 * LOG2E), masked)
            e = jnp.exp2(x - jnp.max(x, axis=-1, keepdims=True))
            total = jnp.sum(e, axis=-1, keepdims=True)
            inv = pltpu.reciprocal(total, approx=True)
            inv = inv * (2.0 - total * inv)
            p_v[j // 4][j % 4] = (e * inv).astype(BF16)

        def attend(j):
            o = _dot(p_v[j // 4][j % 4], stationary(2, j))
            o_v[j // 4][2 * (j % 4)] = o[:L]
            o_v[j // 4][2 * (j % 4) + 1] = o[L:]

        acc = [None] * 4

        def output(g, n):
            lhs = jnp.concatenate([o_v[g // 2][4 * (g % 2) + i] for i in range(4)], axis=1)
            y = _dot(lhs, wo_v[n, 512 * g:512 * g + 512, :])
            acc[n] = y if acc[n] is None else acc[n] + y

        tiles = [(w, head) for g in range(4) for w in (0, 1) for head in range(8 * g, 8 * g + 8)]
        tiles += [(2, head) for head in range(H)]
        stream = [P(qkv_slice, tiles[:4], k) for k in range(4)] + [P(qkv, *t) for t in tiles[4:]]
        stream += [P(output, g, n) for g in range(8) for n in range(3)] + [P(output, g, 3) for g in range(8)]
        trailing = {}
        for g in range(4):
            for j in range(4 * g, 4 * g + 4):
                trailing.setdefault(16 * (g + 1) + 9, []).append(P(scores, j))
            for j in range(4 * g, 4 * g + 4):
                trailing.setdefault(16 * (g + 1) + 12 + 2 * (j % 4), []).append(P(softmax, j))
            for j in range(4 * g, 4 * g + 4):
                trailing.setdefault(64 + 8 * (g + 1) + (6 if g < 3 else 5), []).append(P(attend, j))
        for i, task in enumerate(stream):
            for extra in trailing.get(i, []):
                extra()
            task()
        segment = pl.ds(pl.multiple_of(s * SEG, SEG), SEG)
        for c in range(4):
            out_v[segment, 128 * c:128 * c + 128] = ya_v[c, pl.ds(pl.multiple_of(s * YP, 8), SEG), :].astype(BF16)
            out_v[segment, D + 128 * c:D + 128 * c + 128] = acc[c][M:].astype(BF16)
        return [a[:M] for a in acc]

    def out_copy(s):
        segment = pl.ds(pl.multiple_of(s * SEG, SEG), SEG)
        return pltpu.make_async_copy(out_v.at[segment], out_hbm.at[segment], out_sem)

    def steps(first, count, i, mem):
        for u in range(count):
            mem = step(first + i * count + u, mem)
            out_copy(first + i * count + u).start()
        return mem

    mem0 = mem_v[...].astype(F32)
    mem = [mem0[:, 128 * k:128 * (k + 1)] for k in range(4)]
    odd = NSEG % UNROLL
    mem = lax.fori_loop(0, 1 + zero_ref[0], P(steps, 0, odd), mem)
    lax.fori_loop(0, NSEG // UNROLL, P(steps, odd, UNROLL), mem)

    def drain(s, c):
        out_copy(s).wait()
        return c

    lax.fori_loop(0, NSEG, drain, 0)


@jax.jit
def _forward(A_x, A_w_r, A_w_i, B_x, B_mem0, B_Wq, B_Wk, B_Wv, B_Wo):
    vmem = pltpu.VMEM
    scratch = [
        vmem((S, D), BF16), vmem((D // 2 + 1, S), BF16), vmem((D // 2 + 1, S), BF16), vmem((S, D), BF16),
        vmem((M, D), BF16), vmem((12, D, 8, DH), BF16), vmem((4, H * DH, 128), BF16),
        vmem(_CD.shape, U32), vmem(_G.shape, U32), vmem(_GT.shape, U32), vmem(_TW.shape, F32),
        vmem((A_ROWS, 128), U32), vmem((2, S, 128), U32), vmem((7, 2, R0 // 4, 128), U32),
        vmem((4, R0 // 2, 128), U32), vmem((2, 4, 2 * N2, 128), F32), vmem((2, N1, 2 * N2, 128), F32),
        vmem((N2, 128), F32), vmem((N2, 128), F32), vmem((4, YP * (N2 + 1), 128), F32), vmem((S, 2 * D), BF16),
    ]
    scratch += [vmem((24, RING, DH), F32)] * 4 + [vmem((24, M, DH), F32)] * 4
    scratch += [vmem((4, 2 * L, 128), F32)] * 4 + [vmem((4, 2 * L, 128), BF16)] * 4 + [vmem((8, L, DH), F32)] * 4
    scratch += [pltpu.SemaphoreType.DMA((29,)), pltpu.SemaphoreType.DMA(())]
    out = pl.pallas_call(
        _kernel,
        out_shape=jax.ShapeDtypeStruct((S, 2 * D), BF16),
        in_specs=[pl.BlockSpec(memory_space=pltpu.SMEM)] + [pl.BlockSpec(memory_space=pltpu.HBM)] * 13,
        out_specs=pl.BlockSpec(memory_space=pltpu.HBM),
        scratch_shapes=scratch,
        compiler_params=pltpu.CompilerParams(vmem_limit_bytes=120 * 1024 * 1024),
    )(np.zeros((1,), np.int32), A_x.reshape(S, D), A_w_r.T, A_w_i.T, B_x.reshape(S, D), B_mem0.reshape(M, D),
      B_Wq, B_Wk, B_Wv, B_Wo.reshape(H * DH, D), _CD, _G, _GT, _TW)
    return out.reshape(1, S, 2 * D)


def pallas_concat_heads__spectral_gfnet__memory_aug_recurrent_mem_tr__prompt_kernel(
        A_x, A_w_r, A_w_i, B_x, B_mem0, B_Wq, B_Wk, B_Wv, B_Wo, B_seg_len):
    assert int(B_seg_len) == SEG and A_x.shape == B_x.shape == (1, S, D) and B_Wq.shape == (D, H, DH)
    return _forward(A_x, A_w_r, A_w_i, B_x, B_mem0, B_Wq, B_Wk, B_Wv, B_Wo)
```

```python
import functools

import jax
import jax.numpy as jnp
import numpy as np
from jax import lax
from jax.experimental import pallas as pl
from jax.experimental.pallas import tpu as pltpu

F32, BF16, U32 = jnp.float32, jnp.bfloat16, jnp.uint32
P = functools.partial

S, D = 2048, 512
H, DH, M, SEG = 32, 128, 8, 32
L = M + SEG
NSEG = S // SEG
N1, N2 = 32, 64
R0, RX = 512, 24
RING = 576
UNROLL = 7
XP, YP, TP = 17, 40, 9
LOG2E = 1.4426950408889634

TILE = D // 2
TMP_ROWS = TP * TILE
XP_ROWS = XP * N2 + 24
A_WEIGHTS = 0
A_TMP = A_WEIGHTS + 3 * H * TILE
A_SUMS = A_TMP + 2 * TMP_ROWS + 16
A_XP = A_SUMS + 2 * 5 * 128
A_Y = A_XP + 4 * XP_ROWS
A_ROWS = A_Y + 2 * N1 * 2 * N2


def _pack_bf16(a):
    u = np.ascontiguousarray(a, dtype=np.float32).view(np.uint32)
    b = ((u + 0x7FFF + ((u >> 16) & 1)) >> 16).astype(np.uint32)
    return b[..., 0::2, :] | (b[..., 1::2, :] << 16)


def _dft_constants():
    lane = np.arange(128)
    angle = lambda k: 2 * np.pi * np.outer(lane, k) / D
    even = lane % 2 == 0
    re, im = np.cos(angle(2 * lane)), -np.sin(angle(2 * ((lane - 1) % 128)))
    fa, fb = np.where(even[None, :], re, im), np.where(even[None, :], im, re)
    fa[:, 1] = np.cos(np.pi * lane)
    p, q = np.cos(angle(2 * lane + 1)), -np.sin(angle(2 * lane + 1))
    sign = np.where(even, -1.0, 1.0)[None, :]
    f2, f3 = q - sign * p, p + sign * q
    scale = 2.0 / (S * D)
    once = np.where(lane < 2, 0.5, 1.0)[None, :]
    inverse = [(m * scale).T for m in (fa * once, fb, p, sign * f2, f3)]
    a32 = 2 * np.pi * np.outer(np.arange(N1), np.arange(N1)) / N1
    c32, s32 = np.zeros((128, 128)), np.zeros((128, 128))
    c32[:N1, :N1], s32[:N1, :N1] = np.cos(a32), np.sin(a32)
    model_axis = np.concatenate([fa, fb, p, f2, f3] + inverse + [c32, s32], axis=0)
    k2 = np.arange(N2)
    g = np.zeros((N1, 2 * N2, 2 * N2))
    for n1 in range(N1):
        a = 2 * np.pi * np.outer(k2, n1 + N1 * k2) / S
        g[n1] = np.block([[np.cos(a), np.sin(a)], [-np.sin(a), np.cos(a)]])
    a = 2 * np.pi * np.outer(k2, np.arange(N1)) / S
    twiddle = np.zeros((2, N2, 128), np.float32)
    twiddle[0, :, :N1], twiddle[1, :, :N1] = np.cos(a), np.sin(a)
    return _pack_bf16(model_axis), _pack_bf16(g), _pack_bf16(g.transpose(0, 2, 1)), twiddle


_CD, _G, _GT, _TW = _dft_constants()
_FA, _FB, _F1, _F2, _F3, _IA, _IB, _I1, _I2, _I3, _C32, _S32 = range(12)


def _dot(a, b):
    return jnp.dot(a, b, preferred_element_type=F32)


def _as_bf16(words):
    return pltpu.bitcast(words, BF16)


def _low(words):
    return pltpu.bitcast(words << 16, F32)


def _high(words):
    return pltpu.bitcast(words & jnp.uint32(0xFFFF0000), F32)


def _add(a, b):
    return a[0] + b[0], a[1] + b[1]


def _sub(a, b):
    return a[0] - b[0], a[1] - b[1]


def _add_i(a, b):
    return a[0] - b[1], a[1] + b[0]


def _sub_i(a, b):
    return a[0] + b[1], a[1] - b[0]


def _twiddle(a, e, n):
    e %= n
    if e == 0:
        return a
    if 4 * e == n:
        return a[1], -a[0]
    if 4 * e == 3 * n:
        return -a[1], a[0]
    if 2 * e == n:
        return -a[0], -a[1]
    c, s = float(np.cos(2 * np.pi * e / n)), float(np.sin(2 * np.pi * e / n))
    if (8 * e) % n == 0:
        h = abs(c)
        if c > 0 and s > 0:
            return (a[0] + a[1]) * h, (a[1] - a[0]) * h
        if c < 0 and s > 0:
            return (a[1] - a[0]) * h, (a[0] + a[1]) * (-h)
        if c < 0 and s < 0:
            return (a[0] + a[1]) * (-h), (a[0] - a[1]) * h
        return (a[0] - a[1]) * h, (a[0] + a[1]) * h
    return a[0] * c + a[1] * s, a[1] * c - a[0] * s


def _dft4(z, forward):
    a, b, c, d = _add(z[0], z[2]), _sub(z[0], z[2]), _add(z[1], z[3]), _sub(z[1], z[3])
    if forward:
        return [_add(a, c), _sub_i(b, d), _sub(a, c), _add_i(b, d)]
    return [_add(a, c), _add_i(b, d), _sub(a, c), _sub_i(b, d)]


def _fft8(z):
    ev = _dft4([_add(z[j], z[j + 4]) for j in range(4)], True)
    d = [_sub(z[j], z[j + 4]) for j in range(4)]
    d1, d3 = _twiddle(d[1], 1, 8), _twiddle(d[3], 3, 8)
    a, b, c, e = _sub_i(d[0], d[2]), _add_i(d[0], d[2]), _add(d1, d3), _sub(d1, d3)
    od = [_add(a, c), _sub_i(b, e), _sub(a, c), _add_i(b, e)]
    return [ev[m // 2] if m % 2 == 0 else od[m // 2] for m in range(8)]


def _ifft8(x):
    ev = _dft4([x[0], x[2], x[4], x[6]], False)
    od = _dft4([x[1], x[3], x[5], x[7]], False)
    o1, o3 = _twiddle(od[1], -1, 8), _twiddle(od[3], -3, 8)
    lo = [_add(ev[0], od[0]), _add(ev[1], o1), _add_i(ev[2], od[2]), _add(ev[3], o3)]
    hi = [_sub(ev[0], od[0]), _sub(ev[1], o1), _sub_i(ev[2], od[2]), _sub(ev[3], o3)]
    return lo + hi


def _run(tasks):
    pending = [g for g in (f() for f in tasks) if g is not None and next(g, 0) is None]
    for g in pending:
        next(g, None)


def _kernel(zero_ref, ax_hbm, wr_hbm, wi_hbm, bx_hbm, mem_hbm, wq_hbm, wk_hbm, wv_hbm, wo_hbm,
            cd_hbm, g_hbm, gt_hbm, tw_hbm, out_hbm,
            ax_v, wr_v, wi_v, bx_v, mem_v, w_v, wo_v, cd_v, g_v, gt_v, tw_v,
            arena, filt_v, xsum_v, x_v, e_v, y_v, nyq_in, nyq_out, ya_v, out_v, *rest):
    rings, mems, s_v, p_v, o_v = [rest[4 * i:4 * i + 4] for i in range(5)]
    sems, out_sem = rest[20:]
    pin = pl.multiple_of(zero_ref[0], 8)

    copies = {}

    def add_copy(name, src, dst):
        copies[name] = pltpu.make_async_copy(src, dst, sems.at[len(copies)])

    def wait(*names):
        for name in names:
            copies[name].wait()

    for u in range(1, 12):
        add_copy(u, (wq_hbm, wk_hbm, wv_hbm)[u // 4].at[:, pl.ds(8 * (u % 4), 8), :], w_v.at[u])
    w0 = [("w0", q) for q in range(4)]
    for q in range(4):
        add_copy(w0[q], wq_hbm.at[pl.ds(128 * q, 128), pl.ds(0, 8), :], w_v.at[0, pl.ds(128 * q, 128)])
    add_copy("bx0", bx_hbm.at[pl.ds(0, R0)], bx_v.at[pl.ds(0, R0)])
    add_copy("bx1", bx_hbm.at[pl.ds(R0, S - R0)], bx_v.at[pl.ds(R0, S - R0)])
    wo = [("wo", n) for n in range(4)]
    for n in range(4):
        add_copy(wo[n], wo_hbm.at[:, pl.ds(128 * n, 128)], wo_v.at[n])
    for name, src, dst in (("ax", ax_hbm, ax_v), ("wr", wr_hbm, wr_v), ("wi", wi_hbm, wi_v), ("mem", mem_hbm, mem_v),
                           ("cd", cd_hbm, cd_v), ("g", g_hbm, g_v), ("gt", gt_hbm, gt_v), ("tw", tw_hbm, tw_v)):
        add_copy(name, src, dst)

    lane = lax.broadcasted_iota(jnp.int32, (N2, 128), 1)
    lane2 = lax.broadcasted_iota(jnp.int32, (2 * N2, 128), 1)
    lane_sign = jnp.where((lane2 & 1) == 0, -1.0, 1.0).astype(F32)

    def const(i):
        return _as_bf16(cd_v[64 * i:64 * i + 64, :])

    def tile_row(t):
        return A_WEIGHTS + TILE * t

    def weight(t, lo=0, hi=TILE):
        return _as_bf16(arena[tile_row(t) + lo:tile_row(t) + hi, :])

    def stage(u, piece):
        words = pltpu.bitcast(w_v[u, 32 * piece:32 * piece + 32].reshape(32 * 8, DH), U32)
        yield
        for j in range(16):
            row = A_TMP + (u % 2) * TMP_ROWS + TP * (16 * piece + j)
            arena[pl.ds(pin + row, 8), :] = words[8 * j:8 * j + 8]

    def relayout(pair, k, sums):
        u, i = divmod(pair, 4)
        halves = [[arena[pl.ds(A_TMP + (u % 2) * TMP_ROWS + TP * (128 * half + 16 * k) + i + 4 * q, 16, stride=TP), :]
                   for q in range(2)] for half in range(2)]
        yield
        for half, (ev, od) in enumerate(halves):
            row = (0 if sums else pin) + tile_row(2 * pair) + 128 * half + 16 * k
            arena[pl.ds(row, 16), :] = (ev & jnp.uint32(0xFFFF)) | (od << 16)
            arena[pl.ds(row + TILE, 16), :] = (ev >> 16) | (od & jnp.uint32(0xFFFF0000))
        if sums:
            b11, b12, b21, b22 = [(f(ev), f(od)) for ev, od in halves for f in (_low, _high)]
            for n, t in enumerate((_add(b11, b22), _sub(b12, b22), _sub(b21, b11), _add(b11, b12), _add(b21, b22))):
                ev, od = [pltpu.bitcast(v, U32) + jnp.uint32(0x8000) for v in t]
                arena[pl.ds(pin + A_SUMS + ((pair % 2) * 5 + n) * 128 + 16 * k, 16), :] = (
                    (ev >> 16) | (od & jnp.uint32(0xFFFF0000)))

    def token_sums():
        def quad(r, k):
            return bx_v[256 * r:256 * r + 256, 256 * k:256 * k + 256].astype(F32)

        for k in range(4):
            x_v[k] = pltpu.bitcast(bx_v[0:R0, 128 * k:128 * k + 128], U32)
        a11, a12, a21, a22 = quad(0, 0), quad(0, 1), quad(1, 0), quad(1, 1)
        for i, t in enumerate((a11 + a22, a21 + a22, a11, a22, a11 + a12, a21 - a11, a12 - a22)):
            for k in range(2):
                xsum_v[i, k] = pltpu.bitcast(t[:, 128 * k:128 * k + 128].astype(BF16), U32)

    def put_tokens(t, row, y):
        w, head = divmod(t, H)
        rings[head // 8][8 * w + head % 8, pl.ds(RING - R0 + row, y.shape[0]), :] = y

    def project(t, c):
        lhs = jnp.concatenate([_as_bf16(x_v[k, 64 * c:64 * c + 64, :]) for k in range(4)], axis=1)
        put_tokens(t, 128 * c, _dot(lhs, weight(t)))

    def product(pair, i, c, rows):
        words = slice(rows // 2 * c, rows // 2 * (c + 1))
        lhs = jnp.concatenate([_as_bf16(xsum_v[i - 1, k, words, :]) for k in range(2)], axis=1)
        if i == 2:
            return _dot(lhs, weight(2 * pair, 0, 128))
        if i == 5:
            return _dot(lhs, weight(2 * pair + 1, 128, 256))
        row = A_SUMS + ((pair % 2) * 5 + (1, 3, 4, 6, 7).index(i)) * 128
        return _dot(lhs, _as_bf16(arena[row:row + 128, :]))

    carry = []

    def strassen64(pair, c, part):
        m = lambda i: product(pair, i, c, 64)
        if part == 0:
            m3, m5, m2, m4 = m(3), m(5), m(2), m(4)
            put_tokens(2 * pair + 1, 64 * c, m3 + m5)
            put_tokens(2 * pair, 256 + 64 * c, m2 + m4)
            carry.append((m4 - m5, m3 - m2))
        else:
            t11, t22 = carry.pop()
            m1, m7, m6 = m(1), m(7), m(6)
            put_tokens(2 * pair, 64 * c, m1 + m7 + t11)
            put_tokens(2 * pair + 1, 256 + 64 * c, m1 + m6 + t22)

    def strassen128(pair, c, part):
        m = lambda i: product(pair, i, c, 128)
        if part == 0:
            m3, m5 = m(3), m(5)
            put_tokens(2 * pair + 1, 128 * c, m3 + m5)
            carry.append((m5, m3))
        elif part == 1:
            m5, m3 = carry.pop()
            m2, m4 = m(2), m(4)
            put_tokens(2 * pair, 256 + 128 * c, m2 + m4)
            carry.append((m4 - m5, m3 - m2))
        elif part == 2:
            t11, t22 = carry.pop()
            m1, m7 = m(1), m(7)
            put_tokens(2 * pair, 128 * c, m1 + m7 + t11)
            carry.append(m1 + t22)
        else:
            m6 = m(6)
            put_tokens(2 * pair + 1, 256 + 128 * c, m6 + carry.pop())

    def decimate(n2):
        yield
        for c in range(4):
            arena[pl.ds(pin + A_XP + c * XP_ROWS + XP * n2, 16), :] = pltpu.bitcast(
                ax_v[32 * n2:32 * n2 + 32, 128 * c:128 * c + 128], U32)

    def forward_model_axis(a):
        xs = []
        for c in range(4):
            words = arena[pl.ds(A_XP + c * XP_ROWS + a, N2, stride=XP), :]
            xs.append(jnp.concatenate([_low(words), _high(words)], axis=0))
        u0, u1, v0, v1 = xs[0] + xs[2], xs[1] + xs[3], xs[0] - xs[2], xs[1] - xs[3]
        e_v[a % 2, 0] = _dot(u0 + u1, const(_FA))
        e_v[a % 2, 1] = _dot(u0 - u1, const(_FB))
        k1 = _dot(v0 + v1, const(_F1))
        e_v[a % 2, 2] = k1 - _dot(v1, const(_F3))
        e_v[a % 2, 3] = k1 * lane_sign + _dot(v0, const(_F2))

    def forward_sequence_axis(a, p):
        n1 = 2 * a + p
        ea, eb, ore, oim = [e_v[a % 2, q, N2 * p:N2 * p + N2, :] for q in range(4)]
        even = (lane & 1) == 0
        ere = jnp.where(even, ea, eb)
        eim = pltpu.roll(jnp.where(even, eb, jnp.where(lane == 1, 0.0, ea)), 127, 1)
        nyquist = pltpu.roll(ea, (n1 - 1) % 128, 1) if n1 != 1 else ea
        nyq_in[...] = jnp.where(lane == n1, nyquist, 0.0 if n1 == 0 else nyq_in[...])
        g = _as_bf16(g_v[n1])
        y_v[0, n1] = _dot(g, jnp.concatenate([ere, eim], axis=0).astype(BF16))
        y_v[1, n1] = _dot(g, jnp.concatenate([ore, oim], axis=0).astype(BF16))

    def transpose_filter(q, c):
        filt_v[q, 128 * c:128 * c + 128, :] = pltpu.bitcast((wr_v, wi_v)[q][0:256, 128 * c:128 * c + 128], U32).T

    def spectrum_row(t, n):
        return A_Y + (t * N1 + n) * 2 * N2

    def load(t, n, j):
        row = spectrum_row(t, n) + 8 * j
        return pltpu.bitcast(arena[row:row + 8, :], F32), pltpu.bitcast(arena[row + N2:row + N2 + 8, :], F32)

    def store(t, n, j, z):
        row = spectrum_row(t, n) + 8 * j
        arena[pl.ds(pin + row, 8), :] = pltpu.bitcast(z[0], U32)
        arena[pl.ds(pin + row + N2, 8), :] = pltpu.bitcast(z[1], U32)

    def fft_first(t, j, j1):
        z = [(y_v[t, j1 + 8 * q, 8 * j:8 * j + 8, :], y_v[t, j1 + 8 * q, N2 + 8 * j:N2 + 8 * j + 8, :])
             for q in range(4)]
        o = _dft4(z, True)
        yield
        for r in range(4):
            store(t, 8 * r + j1, j, _twiddle(o[r], r * j1, N1))

    def fft_filter(t, j, r):
        x = _fft8([load(t, 8 * r + j1, j) for j1 in range(8)])
        for m in range(8):
            row = N2 * (4 * m + r) + 8 * j
            fr, fi = [(_low, _high)[t](filt_v[q, row:row + 8, :]) for q in range(2)]
            x[m] = (x[m][0] * fr - x[m][1] * fi, x[m][0] * fi + x[m][1] * fr)
        z = _ifft8(x)
        yield
        for j1 in range(8):
            store(t, 8 * r + j1, j, z[j1])

    def fft_last(t, j, half):
        cols = range(4 * half, 4 * half + 4)
        o = {j1: [load(t, 8 * r + j1, j) for r in range(4)] for j1 in cols}
        yield
        for j1 in cols:
            z = _dft4([_twiddle(o[j1][r], -r * j1, N1) for r in range(4)], False)
            for q in range(4):
                store(t, j1 + 8 * q, j, z[q])

    nyq = []

    def nyquist_1():
        rhs = jnp.concatenate([nyq_in[...], jnp.zeros((N2, 128), F32)], axis=0).astype(BF16)
        nyq.append(_dot(_as_bf16(g_v[0]), rhs))

    def nyquist_2():
        y = nyq.pop()
        c, s = tw_v[0], tw_v[1]
        y = jnp.concatenate([y[:N2] * c + y[N2:] * s, y[N2:] * c - y[:N2] * s], axis=0)
        nyq.append((_dot(y, const(_C32)), _dot(y, const(_S32))))

    def nyquist_filter(ref):
        row = lax.broadcasted_iota(jnp.int32, (N1, 128), 0)
        f = jnp.zeros((N1, 128), F32)
        for c in range(16):
            v = jnp.broadcast_to(ref[256:257, 128 * c:128 * c + 128].astype(F32), (8, 128))
            f = jnp.where(row == 2 * c, jnp.concatenate([v] * 4, axis=0), f)
            f = jnp.where(row == 2 * c + 1, jnp.concatenate([pltpu.roll(v, 64, 1)] * 4, axis=0), f)
        return jnp.concatenate([f, jnp.zeros((128 - N1, 128), F32)], axis=0).T[:N2]

    def nyquist_3():
        yc, ys = nyq.pop()
        xr, xi = yc[:N2] + ys[N2:], yc[N2:] - ys[:N2]
        fr, fi = nyquist_filter(wr_v), nyquist_filter(wi_v)
        x = jnp.concatenate([xr * fr - xi * fi, xr * fi + xi * fr], axis=0)
        nyq.append((_dot(x, const(_C32)), _dot(x, const(_S32))))

    def nyquist_4():
        xc, xs = nyq.pop()
        tr, ti = xc[:N2] - xs[N2:], xc[N2:] + xs[:N2]
        c, s = tw_v[0], tw_v[1]
        t = jnp.concatenate([tr * c - ti * s, ti * c + tr * s], axis=0).astype(BF16)
        nyq_out[...] = _dot(_as_bf16(gt_v[0, 0:N2 // 2, :]), t)

    def inverse_sequence_axis(a, p):
        g = _as_bf16(gt_v[2 * a + p])
        for t in range(2):
            row = spectrum_row(t, 2 * a + p)
            r = _dot(g, pltpu.bitcast(arena[row:row + 2 * N2, :], F32).astype(BF16))
            e_v[a % 2, 2 * t, N2 * p:N2 * p + N2, :] = r[:N2]
            e_v[a % 2, 2 * t + 1, N2 * p:N2 * p + N2, :] = r[N2:]

    def inverse_model_axis(a):
        even = (lane2 & 1) == 0
        ere, eim = e_v[a % 2, 0], pltpu.roll(e_v[a % 2, 1], 1, 1)
        yn = nyq_out[...]
        nyquist = jnp.concatenate([pltpu.roll(yn, (1 - n1) % 128, 1) if n1 != 1 else yn
                                   for n1 in (2 * a, 2 * a + 1)], axis=0)
        ea = _dot(jnp.where(lane2 == 1, nyquist, jnp.where(even, ere, eim)), const(_IA))
        eb = _dot(jnp.where(even, eim, ere), const(_IB))
        ore, oim = e_v[a % 2, 2], e_v[a % 2, 3] * lane_sign
        k1 = _dot(ore + oim, const(_I1))
        v0, v1 = k1 + _dot(oim, const(_I2)), k1 - _dot(ore, const(_I3))
        u0, u1 = ea + eb, ea - eb
        for c, y in enumerate((u0 + v0, u1 + v1, u0 - v0, u1 - v1)):
            for p in range(2):
                ya_v[c, pl.ds(2 * a + p, N2, stride=YP), :] = y[N2 * p:N2 * p + N2]

    main, fast = [], [*range(0, 25), *range(43, 48)]
    for pair in range(48):
        if pair not in fast:
            main += [P(project, 2 * pair + n, c) for n in range(2) for c in range(4)]
        elif 15 <= pair < 21:
            main += [P(strassen128, pair, c, part) for c in range(2) for part in range(4)]
        else:
            main += [P(strassen64, pair, c, part) for c in range(4) for part in range(2)]
    waits = {22: [1], 43: [2], 79: [3, 4], 131: [5, "ax"], 172: [6, "g", "cd"], 203: ["wr", "wi", "tw", 7],
             238: [8, 9], 290: [10, 11, "gt"]}
    side = {slot: [P(wait, *names)] for slot, names in waits.items()}

    def spread(tasks, lo, hi, clear=1):
        free = [i for i in range(lo, hi) if not any(0 <= i - w < clear for w in waits)]
        slots = [free[(j * len(free)) // len(tasks)] for j in range(len(tasks))]
        for slot, task in zip(slots, tasks):
            side.setdefault(slot, []).append(task)
        return slots

    arrival = {name: slot for slot, names in waits.items() for name in names}
    staged = {u: spread([P(stage, u, k + 8 * half) for k in range(8) for half in range(2)],
                        max(arrival[u], 32 * u - 31), 32 * u - 1) for u in range(1, 12)}
    for pair in range(1, 48):
        slots = spread([P(relayout, pair, k, pair in fast) for k in range(8)], 8 * pair - 8, 8 * pair)
        assert pair < 4 or all(staged[pair // 4][2 * k + 1] < slots[k] for k in range(8))
    spread([P(decimate, n2) for n2 in range(N2)], 131, 171)
    tasks = [P(forward_model_axis, 0)]
    for a in range(16):
        tasks += [P(forward_model_axis, a + 1)] if a + 1 < 16 else []
        tasks += [P(forward_sequence_axis, a, 0), P(forward_sequence_axis, a, 1)]
    spread(tasks, 172, 203)
    groups = [(t, j) for j in range(8) for t in range(2)]
    spread([P(transpose_filter, q, c) for c in range(16) for q in range(2)], 203, 230)
    spread([P(fft_first, t, j, j1) for t, j in groups for j1 in range(8)], 204, 238)
    spread([P(fft_filter, t, j, r) for r in range(4) for t, j in groups], 238, 310, clear=2)
    spread([P(fft_last, t, j, half) for t, j in groups for half in range(2)], 310, 343)
    spread([nyquist_1, nyquist_2, nyquist_3], 205, 220)
    spread([nyquist_4], 294, 295)
    tasks = [P(inverse_sequence_axis, 0, 0), P(inverse_sequence_axis, 0, 1)]
    for a in range(16):
        tasks += [P(inverse_sequence_axis, a + 1, 0), P(inverse_sequence_axis, a + 1, 1)] if a + 1 < 16 else []
        tasks += [P(inverse_model_axis, a)]
    spread(tasks, 344, 383)

    for name in ["bx0", *w0, 1, 2, 3, 4, 5, "ax", 6, "g", "cd", "wr", "wi", "tw", 7, 8, 9, 10, 11, "gt", *wo,
                 "bx1", "mem"]:
        copies[name].start()
    wait("bx0")
    token_sums()
    for q in range(4):
        wait(w0[q])
        _run([P(stage, 0, piece) for piece in range(4 * q, 4 * q + 4)])
    for k in range(0, 8, 2):
        _run([P(relayout, 0, k + i, True) for i in range(2)])
    for slot, task in enumerate(main):
        _run(side.get(slot, []))
        task()
    wait(*wo, "bx1", "mem")

    def step(s, mem):
        rows = lax.broadcasted_iota(jnp.int32, (2 * L, 128), 0)
        cols = lax.broadcasted_iota(jnp.int32, (2 * L, 128), 1)
        row = jnp.where(rows >= L, rows - L, rows)
        col = jnp.where(cols >= L, cols - L, cols)
        same_head = ((rows >= L) == (cols >= L)) & (cols < 2 * L)
        visible = same_head & ((row < M) | (row >= col))
        masked = jnp.where(same_head, -1e9 * LOG2E, -jnp.inf).astype(F32)
        xs = bx_v[pl.ds(pl.multiple_of(R0 + s * RX, 8), RX), :].astype(F32)
        write_at = pl.multiple_of((s * RX) % RING, 8)
        read_at = pl.multiple_of((RING - R0 + s * SEG) % RING, SEG)
        hk = [jnp.concatenate([xs[:, 128 * k:128 * (k + 1)], mem[k]], axis=0) for k in range(4)]
        h = jnp.concatenate(hk, axis=1)

        def put(w, head, y):
            mems[head // 8][8 * w + head % 8] = y[RX:]
            rings[head // 8][8 * w + head % 8, pl.ds(write_at, RX), :] = y[:RX]

        def get(w, head):
            return [mems[head // 8][8 * w + head % 8], rings[head // 8][8 * w + head % 8, pl.ds(read_at, SEG), :]]

        def qkv(w, head):
            put(w, head, _dot(h, weight(w * H + head)))

        partial = {}

        def qkv_slice(tiles, k):
            for w, head in tiles:
                y = _dot(hk[k], weight(w * H + head, 64 * k, 64 * k + 64))
                partial[w, head] = y if k == 0 else partial[w, head] + y
                if k == 3:
                    put(w, head, partial.pop((w, head)))

        def stationary(w, j):
            pad = jnp.zeros((128 - 2 * L, DH), F32)
            return jnp.concatenate(get(w, 2 * j) + get(w, 2 * j + 1) + [pad], axis=0).astype(BF16)

        def scores(j):
            q = jnp.concatenate(get(0, 2 * j) + get(0, 2 * j + 1), axis=0)
            s_v[j // 4][j % 4] = lax.dot_general(q, stationary(1, j), (((1,), (1,)), ((), ())),
                                                 preferred_element_type=F32)

        def softmax(j):
            x = jnp.where(visible, s_v[j // 4][j % 4] * (DH ** -0.5 * LOG2E), masked)
            e = jnp.exp2(x - jnp.max(x, axis=-1, keepdims=True))
            total = jnp.sum(e, axis=-1, keepdims=True)
            inv = pltpu.reciprocal(total, approx=True)
            inv = inv * (2.0 - total * inv)
            p_v[j // 4][j % 4] = (e * inv).astype(BF16)

        def attend(j):
            o = _dot(p_v[j // 4][j % 4], stationary(2, j))
            o_v[j // 4][2 * (j % 4)] = o[:L]
            o_v[j // 4][2 * (j % 4) + 1] = o[L:]

        acc = [None] * 4

        def output(g, n):
            lhs = jnp.concatenate([o_v[g // 2][4 * (g % 2) + i] for i in range(4)], axis=1)
            y = _dot(lhs, wo_v[n, 512 * g:512 * g + 512, :])
            acc[n] = y if acc[n] is None else acc[n] + y

        tiles = [(w, head) for g in range(4) for w in (0, 1) for head in range(8 * g, 8 * g + 8)]
        tiles += [(2, head) for head in range(H)]
        stream = [P(qkv_slice, tiles[:4], k) for k in range(4)] + [P(qkv, *t) for t in tiles[4:]]
        stream += [P(output, g, n) for g in range(8) for n in range(3)] + [P(output, g, 3) for g in range(8)]
        trailing = {}
        for g in range(4):
            for j in range(4 * g, 4 * g + 4):
                trailing.setdefault(16 * (g + 1) + 9, []).append(P(scores, j))
            for j in range(4 * g, 4 * g + 4):
                trailing.setdefault(16 * (g + 1) + 12 + 2 * (j % 4), []).append(P(softmax, j))
            for j in range(4 * g, 4 * g + 4):
                trailing.setdefault(64 + 8 * (g + 1) + 6, []).append(P(attend, j))
        for i, task in enumerate(stream):
            for extra in trailing.get(i, []):
                extra()
            task()
        segment = pl.ds(pl.multiple_of(s * SEG, SEG), SEG)
        for c in range(4):
            out_v[segment, 128 * c:128 * c + 128] = ya_v[c, pl.ds(pl.multiple_of(s * YP, 8), SEG), :].astype(BF16)
            out_v[segment, D + 128 * c:D + 128 * c + 128] = acc[c][M:].astype(BF16)
        return [a[:M] for a in acc]

    def out_copy(s):
        segment = pl.ds(pl.multiple_of(s * SEG, SEG), SEG)
        return pltpu.make_async_copy(out_v.at[segment], out_hbm.at[segment], out_sem)

    def steps(first, count, i, mem):
        for u in range(count):
            mem = step(first + i * count + u, mem)
            out_copy(first + i * count + u).start()
        return mem

    mem0 = mem_v[...].astype(F32)
    mem = [mem0[:, 128 * k:128 * (k + 1)] for k in range(4)]
    odd = NSEG % UNROLL
    mem = lax.fori_loop(0, 1 + zero_ref[0], P(steps, 0, odd), mem)
    lax.fori_loop(0, NSEG // UNROLL, P(steps, odd, UNROLL), mem)
    pltpu.make_async_copy(out_v, out_hbm, out_sem).wait()


@jax.jit
def _forward(A_x, A_w_r, A_w_i, B_x, B_mem0, B_Wq, B_Wk, B_Wv, B_Wo):
    vmem = pltpu.VMEM
    scratch = [
        vmem((S, D), BF16), vmem((D // 2 + 1, S), BF16), vmem((D // 2 + 1, S), BF16), vmem((S, D), BF16),
        vmem((M, D), BF16), vmem((12, D, 8, DH), BF16), vmem((4, H * DH, 128), BF16),
        vmem(_CD.shape, U32), vmem(_G.shape, U32), vmem(_GT.shape, U32), vmem(_TW.shape, F32),
        vmem((A_ROWS, 128), U32), vmem((2, S, 128), U32), vmem((7, 2, R0 // 4, 128), U32),
        vmem((4, R0 // 2, 128), U32), vmem((2, 4, 2 * N2, 128), F32), vmem((2, N1, 2 * N2, 128), F32),
        vmem((N2, 128), F32), vmem((N2, 128), F32), vmem((4, YP * (N2 + 1), 128), F32), vmem((S, 2 * D), BF16),
    ]
    scratch += [vmem((24, RING, DH), F32)] * 4 + [vmem((24, M, DH), F32)] * 4
    scratch += [vmem((4, 2 * L, 128), F32)] * 4 + [vmem((4, 2 * L, 128), BF16)] * 4 + [vmem((8, L, DH), F32)] * 4
    scratch += [pltpu.SemaphoreType.DMA((29,)), pltpu.SemaphoreType.DMA(())]
    out = pl.pallas_call(
        _kernel,
        out_shape=jax.ShapeDtypeStruct((S, 2 * D), BF16),
        in_specs=[pl.BlockSpec(memory_space=pltpu.SMEM)] + [pl.BlockSpec(memory_space=pltpu.HBM)] * 13,
        out_specs=pl.BlockSpec(memory_space=pltpu.HBM),
        scratch_shapes=scratch,
        compiler_params=pltpu.CompilerParams(vmem_limit_bytes=120 * 1024 * 1024,
                                             flags={"XLA_TPU_EVENLY_DISTRIBUTE_CRITICAL_NODES": True}),
    )(np.zeros((1,), np.int32), A_x.reshape(S, D), A_w_r.T, A_w_i.T, B_x.reshape(S, D), B_mem0.reshape(M, D),
      B_Wq, B_Wk, B_Wv, B_Wo.reshape(H * DH, D), _CD, _G, _GT, _TW)
    return out.reshape(1, S, 2 * D)


def pallas_concat_heads__spectral_gfnet__memory_aug_recurrent_mem_tr__prompt_kernel(
        A_x, A_w_r, A_w_i, B_x, B_mem0, B_Wq, B_Wk, B_Wv, B_Wo, B_seg_len):
    assert int(B_seg_len) == SEG and A_x.shape == B_x.shape == (1, S, D) and B_Wq.shape == (D, H, DH)
    return _forward(A_x, A_w_r, A_w_i, B_x, B_mem0, B_Wq, B_Wk, B_Wv, B_Wo)
```

```python
import functools

import jax
import jax.numpy as jnp
import numpy as np
from jax import lax
from jax.experimental import pallas as pl
from jax.experimental.pallas import tpu as pltpu

F32, BF16, U32 = jnp.float32, jnp.bfloat16, jnp.uint32
P = functools.partial

S, D = 2048, 512
H, DH, M, SEG = 32, 128, 8, 32
L = M + SEG
NSEG = S // SEG
N1, N2 = 32, 64
R0, RX = 512, 24
RING = 576
UNROLL = 7
XP, YP, TP = 17, 40, 9
LOG2E = 1.4426950408889634

TILE = D // 2
TMP_ROWS = TP * TILE
XP_ROWS = XP * N2 + 24
A_WEIGHTS = 0
A_TMP = A_WEIGHTS + 3 * H * TILE
A_SUMS = A_TMP + 2 * TMP_ROWS + 16
A_XP = A_SUMS + 2 * 5 * 128
A_Y = A_XP + 4 * XP_ROWS
A_ROWS = A_Y + 2 * N1 * 2 * N2


def _pack_bf16(a):
    u = np.ascontiguousarray(a, dtype=np.float32).view(np.uint32)
    b = ((u + 0x7FFF + ((u >> 16) & 1)) >> 16).astype(np.uint32)
    return b[..., 0::2, :] | (b[..., 1::2, :] << 16)


def _dft_constants():
    lane = np.arange(128)
    angle = lambda k: 2 * np.pi * np.outer(lane, k) / D
    even = lane % 2 == 0
    re, im = np.cos(angle(2 * lane)), -np.sin(angle(2 * ((lane - 1) % 128)))
    fa, fb = np.where(even[None, :], re, im), np.where(even[None, :], im, re)
    fa[:, 1] = np.cos(np.pi * lane)
    p, q = np.cos(angle(2 * lane + 1)), -np.sin(angle(2 * lane + 1))
    sign = np.where(even, -1.0, 1.0)[None, :]
    f2, f3 = q - sign * p, p + sign * q
    scale = 2.0 / (S * D)
    once = np.where(lane < 2, 0.5, 1.0)[None, :]
    inverse = [(m * scale).T for m in (fa * once, fb, p, sign * f2, f3)]
    a32 = 2 * np.pi * np.outer(np.arange(N1), np.arange(N1)) / N1
    c32, s32 = np.zeros((128, 128)), np.zeros((128, 128))
    c32[:N1, :N1], s32[:N1, :N1] = np.cos(a32), np.sin(a32)
    model_axis = np.concatenate([fa, fb, p, f2, f3] + inverse + [c32, s32], axis=0)
    k2 = np.arange(N2)
    g = np.zeros((N1, 2 * N2, 2 * N2))
    for n1 in range(N1):
        a = 2 * np.pi * np.outer(k2, n1 + N1 * k2) / S
        g[n1] = np.block([[np.cos(a), np.sin(a)], [-np.sin(a), np.cos(a)]])
    a = 2 * np.pi * np.outer(k2, np.arange(N1)) / S
    twiddle = np.zeros((2, N2, 128), np.float32)
    twiddle[0, :, :N1], twiddle[1, :, :N1] = np.cos(a), np.sin(a)
    return _pack_bf16(model_axis), _pack_bf16(g), _pack_bf16(g.transpose(0, 2, 1)), twiddle


_CD, _G, _GT, _TW = _dft_constants()
_FA, _FB, _F1, _F2, _F3, _IA, _IB, _I1, _I2, _I3, _C32, _S32 = range(12)


def _dot(a, b):
    return jnp.dot(a, b, preferred_element_type=F32)


def _as_bf16(words):
    return pltpu.bitcast(words, BF16)


def _low(words):
    return pltpu.bitcast(words << 16, F32)


def _high(words):
    return pltpu.bitcast(words & jnp.uint32(0xFFFF0000), F32)


def _add(a, b):
    return a[0] + b[0], a[1] + b[1]


def _sub(a, b):
    return a[0] - b[0], a[1] - b[1]


def _add_i(a, b):
    return a[0] - b[1], a[1] + b[0]


def _sub_i(a, b):
    return a[0] + b[1], a[1] - b[0]


def _twiddle(a, e, n):
    e %= n
    if e == 0:
        return a
    if 4 * e == n:
        return a[1], -a[0]
    if 4 * e == 3 * n:
        return -a[1], a[0]
    if 2 * e == n:
        return -a[0], -a[1]
    c, s = float(np.cos(2 * np.pi * e / n)), float(np.sin(2 * np.pi * e / n))
    if (8 * e) % n == 0:
        h = abs(c)
        if c > 0 and s > 0:
            return (a[0] + a[1]) * h, (a[1] - a[0]) * h
        if c < 0 and s > 0:
            return (a[1] - a[0]) * h, (a[0] + a[1]) * (-h)
        if c < 0 and s < 0:
            return (a[0] + a[1]) * (-h), (a[0] - a[1]) * h
        return (a[0] - a[1]) * h, (a[0] + a[1]) * h
    return a[0] * c + a[1] * s, a[1] * c - a[0] * s


def _dft4(z, forward):
    a, b, c, d = _add(z[0], z[2]), _sub(z[0], z[2]), _add(z[1], z[3]), _sub(z[1], z[3])
    if forward:
        return [_add(a, c), _sub_i(b, d), _sub(a, c), _add_i(b, d)]
    return [_add(a, c), _add_i(b, d), _sub(a, c), _sub_i(b, d)]


def _fft8(z):
    ev = _dft4([_add(z[j], z[j + 4]) for j in range(4)], True)
    d = [_sub(z[j], z[j + 4]) for j in range(4)]
    d1, d3 = _twiddle(d[1], 1, 8), _twiddle(d[3], 3, 8)
    a, b, c, e = _sub_i(d[0], d[2]), _add_i(d[0], d[2]), _add(d1, d3), _sub(d1, d3)
    od = [_add(a, c), _sub_i(b, e), _sub(a, c), _add_i(b, e)]
    return [ev[m // 2] if m % 2 == 0 else od[m // 2] for m in range(8)]


def _ifft8(x):
    ev = _dft4([x[0], x[2], x[4], x[6]], False)
    od = _dft4([x[1], x[3], x[5], x[7]], False)
    o1, o3 = _twiddle(od[1], -1, 8), _twiddle(od[3], -3, 8)
    lo = [_add(ev[0], od[0]), _add(ev[1], o1), _add_i(ev[2], od[2]), _add(ev[3], o3)]
    hi = [_sub(ev[0], od[0]), _sub(ev[1], o1), _sub_i(ev[2], od[2]), _sub(ev[3], o3)]
    return lo + hi


def _run(tasks):
    pending = [g for g in (f() for f in tasks) if g is not None and next(g, 0) is None]
    for g in pending:
        next(g, None)


def _kernel(zero_ref, ax_hbm, wr_hbm, wi_hbm, bx_hbm, mem_hbm, wq_hbm, wk_hbm, wv_hbm, wo_hbm,
            cd_hbm, g_hbm, gt_hbm, tw_hbm, out_hbm,
            ax_v, wr_v, wi_v, bx_v, mem_v, w_v, wo_v, cd_v, g_v, gt_v, tw_v,
            arena, filt_v, xsum_v, x_v, e_v, y_v, nyq_in, nyq_out, ya_v, out_v, *rest):
    rings, mems, s_v, p_v, o_v = [rest[4 * i:4 * i + 4] for i in range(5)]
    sems, out_sem = rest[20:]
    pin = pl.multiple_of(zero_ref[0], 8)

    copies = {}

    def add_copy(name, src, dst):
        copies[name] = pltpu.make_async_copy(src, dst, sems.at[len(copies)])

    def wait(*names):
        for name in names:
            copies[name].wait()

    for u in range(1, 12):
        add_copy(u, (wq_hbm, wk_hbm, wv_hbm)[u // 4].at[:, pl.ds(8 * (u % 4), 8), :], w_v.at[u])
    w0 = [("w0", q) for q in range(4)]
    for q in range(4):
        add_copy(w0[q], wq_hbm.at[pl.ds(128 * q, 128), pl.ds(0, 8), :], w_v.at[0, pl.ds(128 * q, 128)])
    add_copy("bx0", bx_hbm.at[pl.ds(0, R0)], bx_v.at[pl.ds(0, R0)])
    add_copy("bx1", bx_hbm.at[pl.ds(R0, S - R0)], bx_v.at[pl.ds(R0, S - R0)])
    wo = [("wo", n) for n in range(4)]
    for n in range(4):
        add_copy(wo[n], wo_hbm.at[:, pl.ds(128 * n, 128)], wo_v.at[n])
    for name, src, dst in (("ax", ax_hbm, ax_v), ("wr", wr_hbm, wr_v), ("wi", wi_hbm, wi_v), ("mem", mem_hbm, mem_v),
                           ("cd", cd_hbm, cd_v), ("g", g_hbm, g_v), ("gt", gt_hbm, gt_v), ("tw", tw_hbm, tw_v)):
        add_copy(name, src, dst)

    lane = lax.broadcasted_iota(jnp.int32, (N2, 128), 1)
    lane2 = lax.broadcasted_iota(jnp.int32, (2 * N2, 128), 1)
    lane_sign = jnp.where((lane2 & 1) == 0, -1.0, 1.0).astype(F32)

    def const(i):
        return _as_bf16(cd_v[64 * i:64 * i + 64, :])

    def tile_row(t):
        return A_WEIGHTS + TILE * t

    def weight(t, lo=0, hi=TILE):
        return _as_bf16(arena[tile_row(t) + lo:tile_row(t) + hi, :])

    def stage(u, piece):
        words = pltpu.bitcast(w_v[u, 32 * piece:32 * piece + 32].reshape(32 * 8, DH), U32)
        yield
        for j in range(16):
            row = A_TMP + (u % 2) * TMP_ROWS + TP * (16 * piece + j)
            arena[pl.ds(pin + row, 8), :] = words[8 * j:8 * j + 8]

    def relayout(pair, k, sums):
        u, i = divmod(pair, 4)
        halves = [[arena[pl.ds(A_TMP + (u % 2) * TMP_ROWS + TP * (128 * half + 16 * k) + i + 4 * q, 16, stride=TP), :]
                   for q in range(2)] for half in range(2)]
        yield
        for half, (ev, od) in enumerate(halves):
            row = (0 if sums else pin) + tile_row(2 * pair) + 128 * half + 16 * k
            arena[pl.ds(row, 16), :] = (ev & jnp.uint32(0xFFFF)) | (od << 16)
            arena[pl.ds(row + TILE, 16), :] = (ev >> 16) | (od & jnp.uint32(0xFFFF0000))
        if sums:
            b11, b12, b21, b22 = [(f(ev), f(od)) for ev, od in halves for f in (_low, _high)]
            for n, t in enumerate((_add(b11, b22), _sub(b12, b22), _sub(b21, b11), _add(b11, b12), _add(b21, b22))):
                ev, od = [pltpu.bitcast(v, U32) + jnp.uint32(0x8000) for v in t]
                arena[pl.ds(pin + A_SUMS + ((pair % 2) * 5 + n) * 128 + 16 * k, 16), :] = (
                    (ev >> 16) | (od & jnp.uint32(0xFFFF0000)))

    def token_sums():
        def quad(r, k):
            return bx_v[256 * r:256 * r + 256, 256 * k:256 * k + 256].astype(F32)

        for k in range(4):
            x_v[k] = pltpu.bitcast(bx_v[0:R0, 128 * k:128 * k + 128], U32)
        a11, a12, a21, a22 = quad(0, 0), quad(0, 1), quad(1, 0), quad(1, 1)
        for i, t in enumerate((a11 + a22, a21 + a22, a11, a22, a11 + a12, a21 - a11, a12 - a22)):
            for k in range(2):
                xsum_v[i, k] = pltpu.bitcast(t[:, 128 * k:128 * k + 128].astype(BF16), U32)

    def put_tokens(t, row, y):
        w, head = divmod(t, H)
        rings[head // 8][8 * w + head % 8, pl.ds(RING - R0 + row, y.shape[0]), :] = y

    def project(t, c):
        lhs = jnp.concatenate([_as_bf16(x_v[k, 64 * c:64 * c + 64, :]) for k in range(4)], axis=1)
        put_tokens(t, 128 * c, _dot(lhs, weight(t)))

    def product(pair, i, c):
        lhs = jnp.concatenate([_as_bf16(xsum_v[i - 1, k, 32 * c:32 * c + 32, :]) for k in range(2)], axis=1)
        if i == 2:
            return _dot(lhs, weight(2 * pair, 0, 128))
        if i == 5:
            return _dot(lhs, weight(2 * pair + 1, 128, 256))
        row = A_SUMS + ((pair % 2) * 5 + (1, 3, 4, 6, 7).index(i)) * 128
        return _dot(lhs, _as_bf16(arena[row:row + 128, :]))

    carry = []

    def strassen(pair, c, part):
        m = lambda i: product(pair, i, c)
        if part == 0:
            m3, m5, m2, m4 = m(3), m(5), m(2), m(4)
            put_tokens(2 * pair + 1, 64 * c, m3 + m5)
            put_tokens(2 * pair, 256 + 64 * c, m2 + m4)
            carry.append((m4 - m5, m3 - m2))
        else:
            t11, t22 = carry.pop()
            m1, m7, m6 = m(1), m(7), m(6)
            put_tokens(2 * pair, 64 * c, m1 + m7 + t11)
            put_tokens(2 * pair + 1, 256 + 64 * c, m1 + m6 + t22)

    def decimate(n2):
        yield
        for c in range(4):
            arena[pl.ds(pin + A_XP + c * XP_ROWS + XP * n2, 16), :] = pltpu.bitcast(
                ax_v[32 * n2:32 * n2 + 32, 128 * c:128 * c + 128], U32)

    def forward_model_axis(a):
        xs = []
        for c in range(4):
            words = arena[pl.ds(A_XP + c * XP_ROWS + a, N2, stride=XP), :]
            xs.append(jnp.concatenate([_low(words), _high(words)], axis=0))
        u0, u1, v0, v1 = xs[0] + xs[2], xs[1] + xs[3], xs[0] - xs[2], xs[1] - xs[3]
        e_v[a % 2, 0] = _dot(u0 + u1, const(_FA))
        e_v[a % 2, 1] = _dot(u0 - u1, const(_FB))
        k1 = _dot(v0 + v1, const(_F1))
        e_v[a % 2, 2] = k1 - _dot(v1, const(_F3))
        e_v[a % 2, 3] = k1 * lane_sign + _dot(v0, const(_F2))

    def forward_sequence_axis(a, p):
        n1 = 2 * a + p
        ea, eb, ore, oim = [e_v[a % 2, q, N2 * p:N2 * p + N2, :] for q in range(4)]
        even = (lane & 1) == 0
        ere = jnp.where(even, ea, eb)
        eim = pltpu.roll(jnp.where(even, eb, jnp.where(lane == 1, 0.0, ea)), 127, 1)
        nyquist = pltpu.roll(ea, (n1 - 1) % 128, 1) if n1 != 1 else ea
        nyq_in[...] = jnp.where(lane == n1, nyquist, 0.0 if n1 == 0 else nyq_in[...])
        g = _as_bf16(g_v[n1])
        y_v[0, n1] = _dot(g, jnp.concatenate([ere, eim], axis=0).astype(BF16))
        y_v[1, n1] = _dot(g, jnp.concatenate([ore, oim], axis=0).astype(BF16))

    def transpose_filter(q, c):
        filt_v[q, 128 * c:128 * c + 128, :] = pltpu.bitcast((wr_v, wi_v)[q][0:256, 128 * c:128 * c + 128], U32).T

    def spectrum_row(t, n):
        return A_Y + (t * N1 + n) * 2 * N2

    def load(t, n, j):
        row = spectrum_row(t, n) + 8 * j
        return pltpu.bitcast(arena[row:row + 8, :], F32), pltpu.bitcast(arena[row + N2:row + N2 + 8, :], F32)

    def store(t, n, j, z):
        row = spectrum_row(t, n) + 8 * j
        arena[pl.ds(pin + row, 8), :] = pltpu.bitcast(z[0], U32)
        arena[pl.ds(pin + row + N2, 8), :] = pltpu.bitcast(z[1], U32)

    def fft_first(t, j, j1):
        z = [(y_v[t, j1 + 8 * q, 8 * j:8 * j + 8, :], y_v[t, j1 + 8 * q, N2 + 8 * j:N2 + 8 * j + 8, :])
             for q in range(4)]
        o = _dft4(z, True)
        yield
        for r in range(4):
            store(t, 8 * r + j1, j, _twiddle(o[r], r * j1, N1))

    def fft_filter(t, j, r):
        x = _fft8([load(t, 8 * r + j1, j) for j1 in range(8)])
        for m in range(8):
            row = N2 * (4 * m + r) + 8 * j
            fr, fi = [(_low, _high)[t](filt_v[q, row:row + 8, :]) for q in range(2)]
            x[m] = (x[m][0] * fr - x[m][1] * fi, x[m][0] * fi + x[m][1] * fr)
        z = _ifft8(x)
        yield
        for j1 in range(8):
            store(t, 8 * r + j1, j, z[j1])

    def fft_last(t, j, half):
        cols = range(4 * half, 4 * half + 4)
        o = {j1: [load(t, 8 * r + j1, j) for r in range(4)] for j1 in cols}
        yield
        for j1 in cols:
            z = _dft4([_twiddle(o[j1][r], -r * j1, N1) for r in range(4)], False)
            for q in range(4):
                store(t, j1 + 8 * q, j, z[q])

    nyq = []

    def nyquist_1():
        rhs = jnp.concatenate([nyq_in[...], jnp.zeros((N2, 128), F32)], axis=0).astype(BF16)
        nyq.append(_dot(_as_bf16(g_v[0]), rhs))

    def nyquist_2():
        y = nyq.pop()
        c, s = tw_v[0], tw_v[1]
        y = jnp.concatenate([y[:N2] * c + y[N2:] * s, y[N2:] * c - y[:N2] * s], axis=0)
        nyq.append((_dot(y, const(_C32)), _dot(y, const(_S32))))

    def nyquist_filter(ref):
        row = lax.broadcasted_iota(jnp.int32, (N1, 128), 0)
        f = jnp.zeros((N1, 128), F32)
        for c in range(16):
            v = jnp.broadcast_to(ref[256:257, 128 * c:128 * c + 128].astype(F32), (8, 128))
            f = jnp.where(row == 2 * c, jnp.concatenate([v] * 4, axis=0), f)
            f = jnp.where(row == 2 * c + 1, jnp.concatenate([pltpu.roll(v, 64, 1)] * 4, axis=0), f)
        return jnp.concatenate([f, jnp.zeros((128 - N1, 128), F32)], axis=0).T[:N2]

    def nyquist_3():
        yc, ys = nyq.pop()
        xr, xi = yc[:N2] + ys[N2:], yc[N2:] - ys[:N2]
        fr, fi = nyquist_filter(wr_v), nyquist_filter(wi_v)
        x = jnp.concatenate([xr * fr - xi * fi, xr * fi + xi * fr], axis=0)
        nyq.append((_dot(x, const(_C32)), _dot(x, const(_S32))))

    def nyquist_4():
        xc, xs = nyq.pop()
        tr, ti = xc[:N2] - xs[N2:], xc[N2:] + xs[:N2]
        c, s = tw_v[0], tw_v[1]
        t = jnp.concatenate([tr * c - ti * s, ti * c + tr * s], axis=0).astype(BF16)
        nyq_out[...] = _dot(_as_bf16(gt_v[0, 0:N2 // 2, :]), t)

    def inverse_sequence_axis(a, p):
        g = _as_bf16(gt_v[2 * a + p])
        for t in range(2):
            row = spectrum_row(t, 2 * a + p)
            r = _dot(g, pltpu.bitcast(arena[row:row + 2 * N2, :], F32).astype(BF16))
            e_v[a % 2, 2 * t, N2 * p:N2 * p + N2, :] = r[:N2]
            e_v[a % 2, 2 * t + 1, N2 * p:N2 * p + N2, :] = r[N2:]

    def inverse_model_axis(a):
        even = (lane2 & 1) == 0
        ere, eim = e_v[a % 2, 0], pltpu.roll(e_v[a % 2, 1], 1, 1)
        yn = nyq_out[...]
        nyquist = jnp.concatenate([pltpu.roll(yn, (1 - n1) % 128, 1) if n1 != 1 else yn
                                   for n1 in (2 * a, 2 * a + 1)], axis=0)
        ea = _dot(jnp.where(lane2 == 1, nyquist, jnp.where(even, ere, eim)), const(_IA))
        eb = _dot(jnp.where(even, eim, ere), const(_IB))
        ore, oim = e_v[a % 2, 2], e_v[a % 2, 3] * lane_sign
        k1 = _dot(ore + oim, const(_I1))
        v0, v1 = k1 + _dot(oim, const(_I2)), k1 - _dot(ore, const(_I3))
        u0, u1 = ea + eb, ea - eb
        for c, y in enumerate((u0 + v0, u1 + v1, u0 - v0, u1 - v1)):
            for p in range(2):
                ya_v[c, pl.ds(2 * a + p, N2, stride=YP), :] = y[N2 * p:N2 * p + N2]

    main, fast = [], [*range(0, 25), *range(43, 48)]
    for pair in range(48):
        if pair in fast:
            main += [P(strassen, pair, c, part) for c in range(4) for part in range(2)]
        else:
            main += [P(project, 2 * pair + n, c) for n in range(2) for c in range(4)]
    waits = {22: [1], 43: [2], 79: [3, 4], 131: [5, "ax"], 172: [6, "g", "cd"], 203: ["wr", "wi", "tw", 7],
             238: [8, 9], 290: [10, 11, "gt"]}
    side = {slot: [P(wait, *names)] for slot, names in waits.items()}

    def spread(tasks, lo, hi, clear=1):
        free = [i for i in range(lo, hi) if not any(0 <= i - w < clear for w in waits)]
        slots = [free[(j * len(free)) // len(tasks)] for j in range(len(tasks))]
        for slot, task in zip(slots, tasks):
            side.setdefault(slot, []).append(task)
        return slots

    arrival = {name: slot for slot, names in waits.items() for name in names}
    staged = {u: spread([P(stage, u, k + 8 * half) for k in range(8) for half in range(2)],
                        max(arrival[u], 32 * u - 31), 32 * u - 1) for u in range(1, 12)}
    for pair in range(1, 48):
        slots = spread([P(relayout, pair, k, pair in fast) for k in range(8)], 8 * pair - 8, 8 * pair)
        assert pair < 4 or all(staged[pair // 4][2 * k + 1] < slots[k] for k in range(8))
    spread([P(decimate, n2) for n2 in range(N2)], 131, 171)
    tasks = [P(forward_model_axis, 0)]
    for a in range(16):
        tasks += [P(forward_model_axis, a + 1)] if a + 1 < 16 else []
        tasks += [P(forward_sequence_axis, a, 0), P(forward_sequence_axis, a, 1)]
    spread(tasks, 172, 203)
    groups = [(t, j) for j in range(8) for t in range(2)]
    spread([P(transpose_filter, q, c) for c in range(16) for q in range(2)], 203, 230)
    spread([P(fft_first, t, j, j1) for t, j in groups for j1 in range(8)], 204, 238)
    spread([P(fft_filter, t, j, r) for r in range(4) for t, j in groups], 238, 310, clear=2)
    spread([P(fft_last, t, j, half) for t, j in groups for half in range(2)], 310, 343)
    spread([nyquist_1, nyquist_2, nyquist_3], 205, 220)
    spread([nyquist_4], 294, 295)
    tasks = [P(inverse_sequence_axis, 0, 0), P(inverse_sequence_axis, 0, 1)]
    for a in range(16):
        tasks += [P(inverse_sequence_axis, a + 1, 0), P(inverse_sequence_axis, a + 1, 1)] if a + 1 < 16 else []
        tasks += [P(inverse_model_axis, a)]
    spread(tasks, 344, 383)

    for name in ["bx0", *w0, 1, 2, 3, 4, 5, "ax", 6, "g", "cd", "wr", "wi", "tw", 7, 8, 9, 10, 11, "gt", *wo,
                 "bx1", "mem"]:
        copies[name].start()
    wait("bx0")
    token_sums()
    for q in range(4):
        wait(w0[q])
        _run([P(stage, 0, piece) for piece in range(4 * q, 4 * q + 4)])
    for k in range(0, 8, 2):
        _run([P(relayout, 0, k + i, True) for i in range(2)])
    for slot, task in enumerate(main):
        _run(side.get(slot, []))
        task()
    wait(*wo, "bx1", "mem")

    def step(s, mem):
        rows = lax.broadcasted_iota(jnp.int32, (2 * L, 128), 0)
        cols = lax.broadcasted_iota(jnp.int32, (2 * L, 128), 1)
        row = jnp.where(rows >= L, rows - L, rows)
        col = jnp.where(cols >= L, cols - L, cols)
        same_head = ((rows >= L) == (cols >= L)) & (cols < 2 * L)
        visible = same_head & ((row < M) | (row >= col))
        masked = jnp.where(same_head, -1e9 * LOG2E, -jnp.inf).astype(F32)
        xs = bx_v[pl.ds(pl.multiple_of(R0 + s * RX, 8), RX), :].astype(F32)
        write_at = pl.multiple_of((s * RX) % RING, 8)
        read_at = pl.multiple_of((RING - R0 + s * SEG) % RING, SEG)
        hk = [jnp.concatenate([xs[:, 128 * k:128 * (k + 1)], mem[k]], axis=0) for k in range(4)]
        h = jnp.concatenate(hk, axis=1)

        def put(w, head, y):
            mems[head // 8][8 * w + head % 8] = y[RX:]
            rings[head // 8][8 * w + head % 8, pl.ds(write_at, RX), :] = y[:RX]

        def get(w, head):
            return [mems[head // 8][8 * w + head % 8], rings[head // 8][8 * w + head % 8, pl.ds(read_at, SEG), :]]

        def qkv(w, head):
            put(w, head, _dot(h, weight(w * H + head)))

        partial = {}

        def qkv_slice(tiles, k):
            for w, head in tiles:
                y = _dot(hk[k], weight(w * H + head, 64 * k, 64 * k + 64))
                partial[w, head] = y if k == 0 else partial[w, head] + y
                if k == 3:
                    put(w, head, partial.pop((w, head)))

        def stationary(w, j):
            pad = jnp.zeros((128 - 2 * L, DH), F32)
            return jnp.concatenate(get(w, 2 * j) + get(w, 2 * j + 1) + [pad], axis=0).astype(BF16)

        def scores(j):
            q = jnp.concatenate(get(0, 2 * j) + get(0, 2 * j + 1), axis=0)
            s_v[j // 4][j % 4] = lax.dot_general(q, stationary(1, j), (((1,), (1,)), ((), ())),
                                                 preferred_element_type=F32)

        def softmax(j):
            x = jnp.where(visible, s_v[j // 4][j % 4] * (DH ** -0.5 * LOG2E), masked)
            e = jnp.exp2(x - jnp.max(x, axis=-1, keepdims=True))
            total = jnp.sum(e, axis=-1, keepdims=True)
            inv = pltpu.reciprocal(total, approx=True)
            inv = inv * (2.0 - total * inv)
            p_v[j // 4][j % 4] = (e * inv).astype(BF16)

        def attend(j):
            o = _dot(p_v[j // 4][j % 4], stationary(2, j))
            o_v[j // 4][2 * (j % 4)] = o[:L]
            o_v[j // 4][2 * (j % 4) + 1] = o[L:]

        acc = [None] * 4

        def output(g, n):
            lhs = jnp.concatenate([o_v[g // 2][4 * (g % 2) + i] for i in range(4)], axis=1)
            y = _dot(lhs, wo_v[n, 512 * g:512 * g + 512, :])
            acc[n] = y if acc[n] is None else acc[n] + y

        tiles = [(w, head) for g in range(4) for w in (0, 1) for head in range(8 * g, 8 * g + 8)]
        tiles += [(2, head) for head in range(H)]
        stream = [P(qkv_slice, tiles[:4], k) for k in range(4)] + [P(qkv, *t) for t in tiles[4:]]
        stream += [P(output, g, n) for g in range(8) for n in range(3)] + [P(output, g, 3) for g in range(8)]
        trailing = {}
        for g in range(4):
            for j in range(4 * g, 4 * g + 4):
                trailing.setdefault(16 * (g + 1) + 9, []).append(P(scores, j))
            for j in range(4 * g, 4 * g + 4):
                trailing.setdefault(16 * (g + 1) + 12 + 2 * (j % 4), []).append(P(softmax, j))
            for j in range(4 * g, 4 * g + 4):
                trailing.setdefault(64 + 8 * (g + 1) + 6, []).append(P(attend, j))
        for i, task in enumerate(stream):
            for extra in trailing.get(i, []):
                extra()
            task()
        segment = pl.ds(pl.multiple_of(s * SEG, SEG), SEG)
        for c in range(4):
            out_v[segment, 128 * c:128 * c + 128] = ya_v[c, pl.ds(pl.multiple_of(s * YP, 8), SEG), :].astype(BF16)
            out_v[segment, D + 128 * c:D + 128 * c + 128] = acc[c][M:].astype(BF16)
        return [a[:M] for a in acc]

    def out_copy(s):
        segment = pl.ds(pl.multiple_of(s * SEG, SEG), SEG)
        return pltpu.make_async_copy(out_v.at[segment], out_hbm.at[segment], out_sem)

    def steps(first, count, i, mem):
        for u in range(count):
            mem = step(first + i * count + u, mem)
            out_copy(first + i * count + u).start()
        return mem

    mem0 = mem_v[...].astype(F32)
    mem = [mem0[:, 128 * k:128 * (k + 1)] for k in range(4)]
    odd = NSEG % UNROLL
    mem = lax.fori_loop(0, 1 + zero_ref[0], P(steps, 0, odd), mem)
    lax.fori_loop(0, NSEG // UNROLL, P(steps, odd, UNROLL), mem)
    pltpu.make_async_copy(out_v, out_hbm, out_sem).wait()


@jax.jit
def _forward(A_x, A_w_r, A_w_i, B_x, B_mem0, B_Wq, B_Wk, B_Wv, B_Wo):
    vmem = pltpu.VMEM
    scratch = [
        vmem((S, D), BF16), vmem((D // 2 + 1, S), BF16), vmem((D // 2 + 1, S), BF16), vmem((S, D), BF16),
        vmem((M, D), BF16), vmem((12, D, 8, DH), BF16), vmem((4, H * DH, 128), BF16),
        vmem(_CD.shape, U32), vmem(_G.shape, U32), vmem(_GT.shape, U32), vmem(_TW.shape, F32),
        vmem((A_ROWS, 128), U32), vmem((2, S, 128), U32), vmem((7, 2, R0 // 4, 128), U32),
        vmem((4, R0 // 2, 128), U32), vmem((2, 4, 2 * N2, 128), F32), vmem((2, N1, 2 * N2, 128), F32),
        vmem((N2, 128), F32), vmem((N2, 128), F32), vmem((4, YP * (N2 + 1), 128), F32), vmem((S, 2 * D), BF16),
    ]
    scratch += [vmem((24, RING, DH), F32)] * 4 + [vmem((24, M, DH), F32)] * 4
    scratch += [vmem((4, 2 * L, 128), F32)] * 4 + [vmem((4, 2 * L, 128), BF16)] * 4 + [vmem((8, L, DH), F32)] * 4
    scratch += [pltpu.SemaphoreType.DMA((29,)), pltpu.SemaphoreType.DMA(())]
    out = pl.pallas_call(
        _kernel,
        out_shape=jax.ShapeDtypeStruct((S, 2 * D), BF16),
        in_specs=[pl.BlockSpec(memory_space=pltpu.SMEM)] + [pl.BlockSpec(memory_space=pltpu.HBM)] * 13,
        out_specs=pl.BlockSpec(memory_space=pltpu.HBM),
        scratch_shapes=scratch,
        compiler_params=pltpu.CompilerParams(vmem_limit_bytes=120 * 1024 * 1024,
                                             flags={"XLA_TPU_EVENLY_DISTRIBUTE_CRITICAL_NODES": True}),
    )(np.zeros((1,), np.int32), A_x.reshape(S, D), A_w_r.T, A_w_i.T, B_x.reshape(S, D), B_mem0.reshape(M, D),
      B_Wq, B_Wk, B_Wv, B_Wo.reshape(H * DH, D), _CD, _G, _GT, _TW)
    return out.reshape(1, S, 2 * D)


def pallas_concat_heads__spectral_gfnet__memory_aug_recurrent_mem_tr__prompt_kernel(
        A_x, A_w_r, A_w_i, B_x, B_mem0, B_Wq, B_Wk, B_Wv, B_Wo, B_seg_len):
    assert A_x.shape == B_x.shape == (1, S, D) and B_mem0.shape == (1, M, D) and B_Wq.shape == (D, H, DH)
    assert not isinstance(B_seg_len, (int, np.integer)) or B_seg_len == SEG
    return _forward(A_x, A_w_r, A_w_i, B_x, B_mem0, B_Wq, B_Wk, B_Wv, B_Wo)
```
